```python
import jax
import jax.numpy as jnp

def _softmax(x, axis=-1):
    return jax.nn.softmax(x, axis=axis)
def _gelu(x):
    return jax.nn.gelu(x, approximate=True)
def _silu(x):
    return jax.nn.silu(x)
def _sigmoid(x):
    return jax.nn.sigmoid(x)
def _layernorm(x, axis=-1, eps=1e-5):
    m = jnp.mean(x, axis=axis, keepdims=True)
    v = jnp.var(x, axis=axis, keepdims=True)
    return (x - m) / jnp.sqrt(v + eps)
def _scatter_add(tgt, idx, src, axis=0):
    return tgt.at[idx].add(src)
def _segment_sum(src, seg, n):
    return jax.ops.segment_sum(src, seg, n)
class _Rng:
    def __init__(self, key):
        self._k = key
    def _next(self):
        self._k, sub = jax.random.split(self._k)
        return sub
    def normal(self, shape):
        return jax.random.normal(self._next(), shape, dtype=jnp.bfloat16)
    def randint(self, lo, hi, shape):
        return jax.random.randint(self._next(), shape, lo, hi, dtype=jnp.int32)
    def uniform(self, shape, lo=0.0, hi=1.0):
        return jax.random.uniform(self._next(), shape, jnp.bfloat16, lo, hi)
    def permutation(self, n):
        return jax.random.permutation(self._next(), n)


kernel_name = 'concat_heads__compressed_kv_cla__sliding_local_dilated__prompt'

def setup_inputs():
    _rng = _Rng(jax.random.key(int.from_bytes(__import__("os").urandom(4), "little")))
    _w = (lambda a: (lambda t: t.astype(jnp.bfloat16) if jnp.issubdtype(t.dtype, jnp.floating) else t)(jnp.asarray(a)))
    def _A_setup():
        B, H, Sq, Sk, D, M = 1, 32, 2048, 2048, 128, 1024
        Dc = 4 * D
        return {
            "x": _w((lambda *s: _rng.normal(s) * 0.05)(B, Sq, M)),
            "c_kv": _w((lambda *s: _rng.normal(s) * 0.05)(B, Sk, Dc)),
            "w_q": _w((lambda *s: _rng.normal(s) * 0.05)(M, H, D) * (M ** -0.5)),
            "w_uk": _w((lambda *s: _rng.normal(s) * 0.05)(Dc, H, D) * (Dc ** -0.5)),
            "w_uv": _w((lambda *s: _rng.normal(s) * 0.05)(Dc, H, D) * (Dc ** -0.5)),
            "w_o": _w((lambda *s: _rng.normal(s) * 0.05)(H, D, M) * ((H * D) ** -0.5)),
        }
    _A_in = _A_setup()

    def _B_setup():
        B, S, D = 1, 2048, 1024
        return {
            "x": _w((lambda *s: _rng.normal(s) * 0.05)(B, S, D)),
            "wqkv": _w((lambda *s: _rng.normal(s) * 0.05)(D, 3 * D)),
            "wo": _w((lambda *s: _rng.normal(s) * 0.05)(D, D)),
        }
    _B_in = _B_setup()

    return {
        "A_x": _A_in["x"],
        "A_c_kv": _A_in["c_kv"],
        "A_w_q": _A_in["w_q"],
        "A_w_uk": _A_in["w_uk"],
        "A_w_uv": _A_in["w_uv"],
        "A_w_o": _A_in["w_o"],
        "B_x": _B_in["x"],
        "B_wqkv": _B_in["wqkv"],
        "B_wo": _B_in["wo"],
    }

def reference(A_x, A_c_kv, A_w_q, A_w_uk, A_w_uv, A_w_o, B_x, B_wqkv, B_wo):
    def _A_ref(x, c_kv, w_q, w_uk, w_uv, w_o):
        B, Sq, M = x.shape[0], x.shape[1], x.shape[2]
        Sk = c_kv.shape[1]
        H, D = w_q.shape[1], w_q.shape[2]
        q = jnp.einsum("bqm,mhd->bhqd", x, w_q)
        k = jnp.einsum("bkc,chd->bhkd", c_kv, w_uk)
        v = jnp.einsum("bkc,chd->bhkd", c_kv, w_uv)
        scores = jnp.einsum("bhqd,bhkd->bhqk", q, k) * (D ** -0.5)
        off = Sk - Sq
        qi = jnp.arange(Sq)[:, None]
        kj = jnp.arange(Sk)[None, :]
        cmask = kj <= (qi + off)
        scores = jnp.where(cmask[None, None], scores, -1e9)
        p = _softmax(scores, axis=-1)
        ctx = jnp.einsum("bhqk,bhkd->bhqd", p, v)
        return jnp.einsum("bhqd,hdm->bqm", ctx, w_o)

    def _B_ref(x, wqkv, wo):
        B, S, D = x.shape
        H = 32; Dh = D // H
        W, dil = 8, 2
        qkv = (lambda x, *d: x.transpose(*d))((x @ wqkv).reshape(B, S, 3, H, Dh), 2, 0, 3, 1, 4)
        q, k, v = qkv[0], qkv[1], qkv[2]
        scale = Dh ** -0.5
        pos = jnp.arange(S)
        off = jnp.arange(W) * dil
        idx = pos[:, None] - off[None, :]
        mask = idx >= 0
        idx_c = jnp.where(mask, idx, 0).reshape(-1)
        kg = k[:, :, idx_c, :].reshape(B, H, S, W, Dh)
        vg = v[:, :, idx_c, :].reshape(B, H, S, W, Dh)
        logits = jnp.einsum("bhsd,bhswd->bhsw", q, kg) * scale
        logits = jnp.where(mask[None, None, :, :], logits, -1e9)
        attn = _softmax(logits, axis=-1)
        o = jnp.einsum("bhsw,bhswd->bhsd", attn, vg)
        return (lambda x, *d: x.transpose(*d))(o, 0, 2, 1, 3).reshape(B, S, D) @ wo

    a = _A_ref(A_x, A_c_kv, A_w_q, A_w_uk, A_w_uv, A_w_o)
    b = _B_ref(B_x, B_wqkv, B_wo)
    return jnp.concatenate([a, b], axis=-1)
```

```python
import math

import jax
import jax.numpy as jnp
from jax import lax
import jax.experimental.pallas as pl
import jax.experimental.pallas.tpu as pltpu

S = 2048
M = 1024
DC = 512
H = 32
D = 128
DH_B = 32
WIN, DIL = 8, 2
HALO = 16

LANES = 128
BQ = 512
CB1 = 512
NRL = 4
BM3 = 256

LOG2E = math.log2(math.e)
NT = (((1,), (1,)), ((), ()))
BF16 = jnp.bfloat16
F32 = jnp.float32


def _dot(a, b):
    return jnp.dot(a, b, preferred_element_type=F32)


def _dot_nt(a, b):
    return lax.dot_general(a, b, NT, preferred_element_type=F32)


def _recip(x):
    r = pltpu.reciprocal(x, approx=True)
    return r * (2.0 - x * r)


def _swap_tile_and_lane_bits(tiles, lane):
    tiles = list(tiles)
    for b in range(3):
        sh = 4 << b
        low = (lane & sh) == 0
        for t in range(8):
            if not t & (1 << b):
                u = t | (1 << b)
                x, y = tiles[t], tiles[u]
                tiles[t] = jnp.where(low, x, pltpu.roll(y, sh, 1))
                tiles[u] = jnp.where(low, pltpu.roll(x, LANES - sh, 1), y)
    return tiles


def _kernel(xa_hbm, c_hbm, wq_hbm, wk_hbm, wv_hbm, woa_hbm, xb_hbm, wqkv_hbm,
            wob_hbm, out_hbm,
            xa, c, wq_raw, wk_raw, wv_raw, wq, wkv, woa, xb, wqkv, wob,
            qkv, ctx, ks, vs, kwin, vwin, oa_buf, ob_buf,
            xb_sem, w1_sem, raw_sem, misc_sem, out_sem):
    ncb = 3 * M // CB1
    xb_rows = ((0, 512), (512, 1024), (1024, 2048))
    rq, rk = M // NRL, DC // NRL

    def xb_copy(i):
        r0, r1 = xb_rows[i]
        return pltpu.make_async_copy(xb_hbm.at[r0:r1], xb.at[r0:r1], xb_sem.at[i])

    def w1_copy(j):
        return pltpu.make_async_copy(
            wqkv_hbm.at[:, pl.ds(j * CB1, CB1)], wqkv.at[j], w1_sem.at[j])

    def raw_copies(i):
        return (
            pltpu.make_async_copy(wk_hbm.at[pl.ds(i * rk, rk)],
                                  wk_raw.at[pl.ds(i * rk, rk)], raw_sem.at[3 * i]),
            pltpu.make_async_copy(wv_hbm.at[pl.ds(i * rk, rk)],
                                  wv_raw.at[pl.ds(i * rk, rk)], raw_sem.at[3 * i + 1]),
            pltpu.make_async_copy(wq_hbm.at[pl.ds(i * rq, rq)],
                                  wq_raw.at[pl.ds(i * rq, rq)], raw_sem.at[3 * i + 2]),
        )

    misc = [pltpu.make_async_copy(src, dst, misc_sem.at[i]) for i, (src, dst) in
            enumerate(((c_hbm, c), (xa_hbm, xa), (woa_hbm, woa), (wob_hbm, wob)))]

    def project_b(j, r0, r1):
        y = _dot(xb[r0:r1, :], wqkv[j])
        qkv[j, HALO + r0:HALO + r1, :] = y.astype(BF16)

    def split_heads(raw, dst, row0, nrows, col0):
        for r in range(0, nrows, 64):
            rows = pl.ds(pl.multiple_of(row0 + r, 64), 64)
            w = raw[rows].reshape(64, H * D)
            for h in range(H):
                dst[h, rows, col0:col0 + D] = w[:, h * D:(h + 1) * D]

    xb_copy(0).start()
    w1_copy(0).start()
    for j in range(M // CB1, ncb):
        qkv[j, 0:HALO, :] = jnp.zeros((HALO, CB1), BF16)
    xb_copy(0).wait()
    w1_copy(0).wait()
    xb_copy(1).start()
    xb_copy(2).start()
    project_b(0, *xb_rows[0])
    xb_copy(1).wait()
    for j in range(1, ncb - NRL + 1):
        w1_copy(j).start()
    project_b(0, *xb_rows[1])
    xb_copy(2).wait()
    for cp in raw_copies(0):
        cp.start()
    project_b(0, *xb_rows[2])
    for j in range(1, ncb - NRL):
        w1_copy(j).wait()
        if j == 1:
            for i in range(1, NRL):
                w1_copy(ncb - NRL + i).start()
                for cp in raw_copies(i):
                    cp.start()
        for r in range(0, S, 512):
            project_b(j, r, r + 512)
    for cp in misc:
        cp.start()

    def phase1_step(i, carry):
        j = ncb - NRL + i
        w1_copy(j).wait()
        for cp in raw_copies(i):
            cp.wait()
        split_heads(wk_raw, wkv, i * rk, rk, 0)
        split_heads(wv_raw, wkv, i * rk, rk, D)
        split_heads(wq_raw, wq, i * rq, rq, 0)
        for r in range(0, S, 512):
            project_b(j, r, r + 512)
        return carry

    lax.fori_loop(0, NRL, phase1_step, 0)
    misc[0].wait()
    misc[1].wait()

    q_scale = D ** -0.5 * LOG2E

    def head_step(h, carry):
        row = lax.broadcasted_iota(jnp.int32, (LANES, LANES), 0)
        col = lax.broadcasted_iota(jnp.int32, (LANES, LANES), 1)
        causal = col <= row
        for r in range(0, S, 512):
            kv = _dot(c[r:r + 512, :], wkv[h])
            ks[r:r + 512, :] = kv[:, :D].astype(BF16)
            vs[r:r + 512, :] = kv[:, D:].astype(BF16)
        nt = BQ // LANES
        for r0 in range(S - BQ, -1, -BQ):
            q = _dot(xa[r0:r0 + BQ, :], wq[h]) * q_scale
            strips = [slice(a * LANES, (a + 1) * LANES) for a in range(nt)]
            s = [[] for _ in range(nt)]
            if r0:
                past = _dot_nt(q.astype(BF16), ks[0:r0, :])
                for a in range(nt):
                    s[a].append(past[strips[a]])
            for a in range(nt):
                near = _dot_nt(q[strips[a]].astype(BF16),
                               ks[r0:r0 + (a + 1) * LANES, :])
                if a:
                    s[a].append(near[:, :a * LANES])
                s[a].append(jnp.where(causal, near[:, a * LANES:], -1e30))
            p, inv = [], []
            for a in range(nt):
                sa = jnp.concatenate(s[a], axis=1)
                pa = jnp.exp2(sa - jnp.max(sa, axis=1, keepdims=True))
                inv.append(_recip(jnp.sum(pa, axis=1, keepdims=True)))
                p.append(pa)
            if r0:
                p_past = jnp.concatenate([pa[:, :r0] for pa in p], axis=0)
                o_past = _dot(p_past.astype(BF16), vs[0:r0, :])
            for a in range(nt):
                o = _dot(p[a][:, r0:].astype(BF16), vs[r0:r0 + (a + 1) * LANES, :])
                if r0:
                    o = o + o_past[strips[a]]
                ctx[h, r0 + a * LANES:r0 + (a + 1) * LANES, :] = (
                    o * inv[a]).astype(BF16)
        return carry

    lax.fori_loop(0, H, head_step, 0)
    misc[2].wait()
    misc[3].wait()

    nblk = S // BM3
    b_scale = DH_B ** -0.5 * LOG2E
    per_part = M // CB1

    def out_copies(i, slot):
        rows = pl.ds(pl.multiple_of(i * BM3, BM3), BM3)
        return (
            pltpu.make_async_copy(oa_buf.at[slot], out_hbm.at[rows, 0:M],
                                  out_sem.at[2 * slot]),
            pltpu.make_async_copy(ob_buf.at[slot], out_hbm.at[rows, M:2 * M],
                                  out_sem.at[2 * slot + 1]),
        )

    def load_part(part, row0, nrows):
        lane = lax.broadcasted_iota(jnp.int32, (nrows, LANES), 1)
        rows = pl.ds(pl.multiple_of(row0, HALO), nrows)
        tiles = []
        for j in range(part * per_part, (part + 1) * per_part):
            y = qkv[j, rows, :].astype(F32)
            tiles += [y[:, t:t + LANES] for t in range(0, CB1, LANES)]
        return _swap_tile_and_lane_bits(tiles, lane)

    def window_attention(r0, a, n):
        lane = lax.broadcasted_iota(jnp.int32, (n, LANES), 1)
        pos = r0 + a + lax.broadcasted_iota(jnp.int32, (n, LANES), 0)
        q = load_part(0, r0 + HALO + a, n)
        logits = []
        for w in range(WIN):
            src = pl.ds(HALO + a - DIL * w, n)
            l = q[0] * kwin[0, src, :]
            for t in range(1, 8):
                l = l + q[t] * kwin[t, src, :]
            for sh in (1, 2):
                l = l + jnp.where((lane & sh) == 0, pltpu.roll(l, LANES - sh, 1),
                                  pltpu.roll(l, sh, 1))
            l = l * b_scale
            if DIL * w > a:
                l = jnp.where(pos >= DIL * w, l, -1e30)
            logits.append(l)
        m = logits[0]
        for l in logits[1:]:
            m = jnp.maximum(m, l)
        e = [jnp.exp2(l - m) for l in logits]
        total = e[0]
        for x in e[1:]:
            total = total + x
        inv = _recip(total)
        e = [x * inv for x in e]
        o = []
        for t in range(8):
            acc = e[0] * vwin[t, pl.ds(HALO + a, n), :]
            for w in range(1, WIN):
                acc = acc + e[w] * vwin[t, pl.ds(HALO + a - DIL * w, n), :]
            o.append(acc)
        return jnp.concatenate(_swap_tile_and_lane_bits(o, lane), axis=1)

    def out_step(i, carry):
        slot = i % 2
        r0 = i * BM3

        @pl.when(i >= 2)
        def _():
            for cp in out_copies(i - 2, slot):
                cp.wait()

        for a in range(0, BM3 + HALO, HALO):
            for part, dst in ((1, kwin), (2, vwin)):
                for t, y in enumerate(load_part(part, r0 + a, HALO)):
                    dst[t, a:a + HALO, :] = y
        rows = pl.ds(pl.multiple_of(r0, BM3), BM3)
        heads = jnp.concatenate([ctx[h, rows, :] for h in range(H)], axis=1)
        oa_buf[slot] = _dot(heads, woa[...]).astype(BF16)
        o = jnp.concatenate(
            [window_attention(r0, a, 16) for a in range(0, BM3, 16)], axis=0)
        ob_buf[slot] = _dot(o.astype(BF16), wob[...]).astype(BF16)
        for cp in out_copies(i, slot):
            cp.start()
        return carry

    lax.fori_loop(0, nblk, out_step, 0)
    for i in (nblk - 2, nblk - 1):
        for cp in out_copies(i, i % 2):
            cp.wait()


@jax.jit
def pallas_concat_heads__compressed_kv_cla__sliding_local_dilated__prompt_kernel(
    A_x: jax.Array,
    A_c_kv: jax.Array,
    A_w_q: jax.Array,
    A_w_uk: jax.Array,
    A_w_uv: jax.Array,
    A_w_o: jax.Array,
    B_x: jax.Array,
    B_wqkv: jax.Array,
    B_wo: jax.Array,
):
    ncb = 3 * M // CB1
    vmem = pltpu.VMEM
    out = pl.pallas_call(
        _kernel,
        out_shape=jax.ShapeDtypeStruct((S, 2 * M), BF16),
        in_specs=[pl.BlockSpec(memory_space=pl.ANY)] * 9,
        out_specs=pl.BlockSpec(memory_space=pl.ANY),
        scratch_shapes=[
            vmem((S, M), BF16),
            vmem((S, DC), BF16),
            vmem((M, H, D), BF16),
            vmem((DC, H, D), BF16),
            vmem((DC, H, D), BF16),
            vmem((H, M, D), BF16),
            vmem((H, DC, 2 * D), BF16),
            vmem((H * D, M), BF16),
            vmem((S, M), BF16),
            vmem((ncb, M, CB1), BF16),
            vmem((M, M), BF16),
            vmem((ncb, HALO + S, CB1), BF16),
            vmem((H, S, D), BF16),
            vmem((S, D), BF16),
            vmem((S, D), BF16),
            vmem((8, HALO + BM3, LANES), F32),
            vmem((8, HALO + BM3, LANES), F32),
            vmem((2, BM3, M), BF16),
            vmem((2, BM3, M), BF16),
            pltpu.SemaphoreType.DMA((3,)),
            pltpu.SemaphoreType.DMA((ncb,)),
            pltpu.SemaphoreType.DMA((3 * NRL,)),
            pltpu.SemaphoreType.DMA((4,)),
            pltpu.SemaphoreType.DMA((4,)),
        ],
        compiler_params=pltpu.CompilerParams(vmem_limit_bytes=120 * 2**20),
        name="fused_attn",
    )(
        A_x.reshape(S, M), A_c_kv.reshape(S, DC), A_w_q, A_w_uk, A_w_uv,
        A_w_o.reshape(H * D, M), B_x.reshape(S, M), B_wqkv, B_wo,
    )
    return out.reshape(1, S, 2 * M)
```

```python
import math

import jax
import jax.numpy as jnp
import numpy as np
from jax import lax
import jax.experimental.pallas as pl
import jax.experimental.pallas.tpu as pltpu

S = 2048
M = 1024
DC = 512
H = 32
D = 128
DH_B = 32
WIN, DIL = 8, 2
HALO = 16

LANES = 128
NTILE = M // LANES
BQ = 512
PM = 256
BM3 = 256
WROWS = M + 2 * DC
WPITCH = WROWS + 1
HPI = 1
WN = 16
PK3 = 4096
FRAC3 = 0.9
KVM = 512
CHAIN = True
KVORD = 0
PIN = 1

LOG2E = math.log2(math.e)
NT = (((1,), (1,)), ((), ()))
BF16 = jnp.bfloat16
F32 = jnp.float32
U32 = jnp.uint32


def _dot(a, b):
    return jnp.dot(a, b, preferred_element_type=F32)


def _dot_nt(a, b):
    return lax.dot_general(a, b, NT, preferred_element_type=F32)


def _recip(x):
    r = pltpu.reciprocal(x, approx=True)
    return r * (2.0 - x * r)


def _ds(start, size, align):
    if not isinstance(start, int):
        start = pl.multiple_of(start, align)
    return pl.ds(start, size)


def _interleave(main, side, frac=1.0):
    done = 0
    for i, f in enumerate(main):
        f()
        upto = min(len(side), int((i + 1) * len(side) / (len(main) * frac)))
        while done < upto:
            side[done]()
            done += 1


def _kernel(xa_hbm, c_hbm, wq_hbm, wk_hbm, wv_hbm, woa_hbm, xb_hbm, wqkv_hbm,
            wob_hbm, out_hbm,
            xa, c, w_raw, w_pair, woa, xb, wqkv, wkv_p, wob, wob_tmp, wob_p,
            qb, qb_p, kvb, tr_tmp, ctx, ks, vs, att, oa_buf, ob_buf,
            in_sem, out_sem):
    nstep = 4
    rr = WROWS // nstep

    def xb_copy(i):
        rows = _ds(i * 512, 512, 512)
        return pltpu.make_async_copy(xb_hbm.at[rows], xb.at[rows], in_sem.at[i])

    wq_b = [pltpu.make_async_copy(wqkv_hbm.at[:, c0:c0 + 512], wqkv.at[:, c0:c0 + 512],
                                  in_sem.at[4 + c0 // 512]) for c0 in (0, 512)]

    def wb_copies(i):
        rows = _ds(i * 512, 512, 512)
        return [
            pltpu.make_async_copy(wqkv_hbm.at[rows, M:3 * M], wqkv.at[rows, M:3 * M],
                                  in_sem.at[6 + i]),
            pltpu.make_async_copy(wob_hbm.at[rows], wob.at[rows], in_sem.at[8 + i])]

    raw_src = (wq_hbm.at[0:rr * H], wq_hbm.at[rr * H:2 * rr * H], wk_hbm, wv_hbm)
    raw = [pltpu.make_async_copy(src, w_raw.at[i], in_sem.at[10 + i])
           for i, src in enumerate(raw_src)]
    misc = [pltpu.make_async_copy(src, dst, in_sem.at[14 + i]) for i, (src, dst) in
            enumerate(((c_hbm, c), (xa_hbm, xa), (woa_hbm, woa)))]
    for cp in ([wq_b[0]] + [xb_copy(i) for i in range(4)] + [wq_b[1]] +
               wb_copies(0) + wb_copies(1) + raw + misc):
        cp.start()

    def to_d_major(load, store):
        def scatter(t):
            ut = pltpu.bitcast(load(t), U32).T
            for j in range(LANES // DH_B):
                tr_tmp[pl.ds(4 * t + j, DH_B, stride=H + 1), :] = (
                    ut[j * DH_B:(j + 1) * DH_B])

        def gather(t):
            v = jnp.concatenate(
                [tr_tmp[pl.ds((4 * t + j) * (H + 1), H), :] for j in range(4)], axis=0)
            store(t, v.T)
        return ([lambda t=t: scatter(t) for t in range(NTILE)] +
                [lambda t=t: gather(t) for t in range(NTILE)])

    def permute_w(part, r):
        def store(t, v):
            wkv_p[part * NTILE + t, _ds(r // 2, LANES, LANES), :] = v
        c0 = (1 + part) * M
        return to_d_major(
            lambda t: wqkv[_ds(r, 256, 256), c0 + t * LANES:c0 + (t + 1) * LANES], store)

    def permute_q(r):
        def store(t, v):
            qb_p[t, _ds(r // 2, LANES, LANES), :] = v
        return to_d_major(lambda t: qb[t, _ds(r, 256, 256), :], store)

    def q_pieces(row0, nrows, tiles):
        def project(r, t):
            rows = _ds(row0 + r, PM, PM)
            y = _dot(xb[rows, :], wqkv[:, t * LANES:(t + 1) * LANES])
            qb[t, rows, :] = y.astype(BF16)
        return [lambda r=r, t=t: project(r, t)
                for r in range(0, nrows, PM) for t in range(*tiles)]

    for t in range(2 * NTILE):
        kvb[t, 0:HALO, :] = jnp.zeros((HALO, LANES), F32)
    wq_b[0].wait()

    def q_step_a(i, carry):
        xb_copy(i).wait()
        _interleave(q_pieces(i * 512, 512, (0, 4)), [])
        return carry

    lax.fori_loop(0, 4, q_step_a, 0)
    wq_b[1].wait()

    def q_step_b(i, carry):
        for cp in wb_copies(i):
            cp.wait()

        def scatter_wob(h):
            y = wob[_ds(h * DH_B, DH_B, DH_B), :].astype(F32)
            for t in range(NTILE):
                wob_tmp[t, pl.ds(h, DH_B, stride=H + 1), :] = (
                    y[:, t * LANES:(t + 1) * LANES])

        side = []
        for part in range(2):
            for r in (0, 256):
                side += permute_w(part, i * 512 + r)
                side += [lambda j=j: scatter_wob(i * 16 + j)
                         for j in range(8 * part + r // 64, 8 * part + r // 64 + 4)]
        _interleave(q_pieces(i * 1024, 1024, (4, 8)), side)
        return carry

    lax.fori_loop(0, 2, q_step_b, 0)

    def kv_step(i, carry):
        pltpu.make_async_copy(wk_hbm, w_raw.at[i], in_sem.at[10 + i]).wait()

        last = []
        never = jnp.full((H // 2, LANES), i) < 0

        def project(r, t):
            w = pltpu.bitcast(wkv_p[4 * i + t], BF16)
            y = _dot(xb[r:r + PM, :], w)
            kvb[4 * i + t, HALO + r:HALO + r + PM, :] = y
            last[:] = [pltpu.bitcast(y[0:H // 2], U32)]

        def split_pairs(r):
            v = pltpu.bitcast(w_raw[i, r * H:(r + 16) * H, :], U32)
            for m in range(16):
                w_pair[pl.ds(i * rr + r + m, H // 2, stride=WPITCH), :] = (
                    jnp.where(never, last[0], v[m * H // 2:(m + 1) * H // 2])
                    if (PIN == 1 or (PIN == 2 and m == 0)) else v[m * H // 2:(m + 1) * H // 2])

        def gather_wob(d):
            wob_p[_ds(d * H, H, H), :] = jnp.concatenate(
                [wob_tmp[t, pl.ds(d * (H + 1), H), :] for t in range(NTILE)],
                axis=1).astype(BF16)

        main = [lambda r=r, t=t: project(r, t)
                for r in range(0, S, PM) for t in range(4)]
        a = [lambda r=r: split_pairs(r) for r in range(0, rr, 16)]
        b = permute_q(i * 512) + permute_q(i * 512 + 256)
        e = [lambda j=j: gather_wob(i * 8 + j) for j in range(8)]
        side = []
        if KVORD == 0:
            for j in range(len(a)):
                side += [a[j], b[j]] + ([e[j // 4]] if j % 4 == 0 else [])
        elif KVORD == 1:
            side = a + b + e
        elif KVORD == 2:
            side = b + e + a
        elif KVORD == 3:
            side = e + b + a
        _interleave(main, side)
        return carry

    lax.fori_loop(0, nstep, kv_step, 0)
    misc[0].wait()
    misc[1].wait()

    q_scale = D ** -0.5 * LOG2E

    def head(pair, odd):
        h = 2 * pair + odd

        def weight(row0, nrows):
            u = w_pair[pl.ds(pair * WPITCH + row0, nrows), :]
            if isinstance(odd, int):
                u = u & np.uint32(0xFFFF0000) if odd else u << 16
            else:
                u = (u << (16 - 16 * odd).astype(U32)) & np.uint32(0xFFFF0000)
            return pltpu.bitcast(u, F32)

        row = lax.broadcasted_iota(jnp.int32, (LANES, LANES), 0)
        col = lax.broadcasted_iota(jnp.int32, (LANES, LANES), 1)
        causal = col <= row
        wkv = jnp.concatenate([weight(M, DC), weight(M + DC, DC)], axis=1).astype(BF16)
        for r in range(0, S, KVM):
            kv = _dot(c[r:r + KVM, :], wkv)
            ks[r:r + KVM, :] = kv[:, :D].astype(BF16)
            vs[r:r + KVM, :] = kv[:, D:].astype(BF16)
        wq = weight(0, M).astype(BF16)
        nt = BQ // LANES
        for r0 in range(S - BQ, -1, -BQ):
            q = _dot(xa[r0:r0 + BQ, :], wq) * q_scale
            strips = [slice(a * LANES, (a + 1) * LANES) for a in range(nt)]
            s = [[] for _ in range(nt)]
            if r0:
                past = _dot_nt(q.astype(BF16), ks[0:r0, :])
                for a in range(nt):
                    s[a].append(past[strips[a]])
            for a in range(nt):
                near = _dot_nt(q[strips[a]].astype(BF16),
                               ks[r0:r0 + (a + 1) * LANES, :])
                if a:
                    s[a].append(near[:, :a * LANES])
                s[a].append(jnp.where(causal, near[:, a * LANES:], -1e30))
            p, inv = [], []
            for a in range(nt):
                sa = jnp.concatenate(s[a], axis=1)
                pa = jnp.exp2(sa - jnp.max(sa, axis=1, keepdims=True))
                inv.append(_recip(jnp.sum(pa, axis=1, keepdims=True)))
                p.append(pa)
            if r0:
                p_past = jnp.concatenate([pa[:, :r0] for pa in p], axis=0)
                o_past = _dot(p_past.astype(BF16), vs[0:r0, :])
            for a in range(nt):
                o = _dot(p[a][:, r0:].astype(BF16), vs[r0:r0 + (a + 1) * LANES, :])
                if r0:
                    o = o + o_past[strips[a]]
                ctx[h, r0 + a * LANES:r0 + (a + 1) * LANES, :] = (
                    o * inv[a]).astype(BF16)

    def head_step(i, carry):
        if HPI == 2:
            head(i, 0)
            head(i, 1)
        else:
            head(i // 2, i % 2)
        return carry

    lax.fori_loop(0, H // HPI, head_step, 0)
    misc[2].wait()

    nblk = S // BM3
    b_scale = DH_B ** -0.5 * LOG2E

    def out_copies(i, slot):
        rows = _ds(i * BM3, BM3, BM3)
        return (
            pltpu.make_async_copy(oa_buf.at[slot], out_hbm.at[rows, 0:M],
                                  out_sem.at[2 * slot]),
            pltpu.make_async_copy(ob_buf.at[slot], out_hbm.at[rows, M:2 * M],
                                  out_sem.at[2 * slot + 1]),
        )

    def window_attention(r0, a, n, prev):
        pos = r0 + a + lax.broadcasted_iota(jnp.int32, (n, LANES), 0)
        q = [pltpu.bitcast(qb_p[t, _ds((r0 + a) // 2, n // 2, 8), :], BF16).astype(F32)
             for t in range(NTILE)]
        if prev and CHAIN:
            q[0] = jnp.where(pos < 0, prev.pop(), q[0])
        src = [pl.ds(r0 + HALO + a - DIL * w, n) for w in range(WIN)]
        logits = []
        for w in range(WIN):
            l = q[0] * kvb[0, src[w], :]
            for t in range(1, NTILE):
                l = l + q[t] * kvb[t, src[w], :]
            l = l + pltpu.roll(l, 2 * H, 1)
            l = (l + pltpu.roll(l, H, 1)) * b_scale
            if DIL * w > a:
                l = jnp.where(pos >= DIL * w, l, -1e30)
            logits.append(l)
        m = logits[0]
        for l in logits[1:]:
            m = jnp.maximum(m, l)
        e = [jnp.exp2(l - m) for l in logits]
        total = e[0]
        for x in e[1:]:
            total = total + x
        inv = _recip(total)
        e = [x * inv for x in e]
        o = []
        for t in range(NTILE):
            acc = e[0] * kvb[NTILE + t, src[0], :]
            for w in range(1, WIN):
                acc = acc + e[w] * kvb[NTILE + t, src[w], :]
            o.append(acc)
        att[a:a + n, :] = jnp.concatenate(o, axis=1).astype(BF16)
        prev.append(o[-1])

    def out_step(i, carry):
        slot = i % 2
        r0 = pl.multiple_of(i * BM3, BM3)

        @pl.when(i >= 2)
        def _():
            for cp in out_copies(i - 2, slot):
                cp.wait()

        acc = {}
        prev = []

        def project_a(n, k):
            heads = jnp.concatenate(
                [ctx[h, pl.ds(r0, BM3), :] for h in range(k // D, (k + PK3) // D)], axis=1)
            y = _dot(heads, woa[k:k + PK3, n:n + LANES])
            acc[n] = y if k == 0 else acc[n] + y
            if k + PK3 == H * D:
                oa_buf[slot, :, n:n + LANES] = acc[n].astype(BF16)

        _interleave(
            [lambda n=n, k=k: project_a(n, k)
             for n in range(0, M, LANES) for k in range(0, H * D, PK3)],
            [lambda a=a: window_attention(r0, a, WN, prev) for a in range(0, BM3, WN)],
            FRAC3)
        for n in range(0, M, LANES):
            ob_buf[slot, :, n:n + LANES] = _dot(
                att[...], wob_p[:, n:n + LANES]).astype(BF16)
        for cp in out_copies(i, slot):
            cp.start()
        return carry

    lax.fori_loop(0, nblk, out_step, 0)
    for i in (nblk - 2, nblk - 1):
        for cp in out_copies(i, i % 2):
            cp.wait()


@jax.jit
def pallas_concat_heads__compressed_kv_cla__sliding_local_dilated__prompt_kernel(
    A_x: jax.Array,
    A_c_kv: jax.Array,
    A_w_q: jax.Array,
    A_w_uk: jax.Array,
    A_w_uv: jax.Array,
    A_w_o: jax.Array,
    B_x: jax.Array,
    B_wqkv: jax.Array,
    B_wo: jax.Array,
):
    vmem = pltpu.VMEM
    out = pl.pallas_call(
        _kernel,
        out_shape=jax.ShapeDtypeStruct((S, 2 * M), BF16),
        in_specs=[pl.BlockSpec(memory_space=pl.ANY)] * 9,
        out_specs=pl.BlockSpec(memory_space=pl.ANY),
        scratch_shapes=[
            vmem((S, M), BF16),
            vmem((S, DC), BF16),
            vmem((4, WROWS // 4 * H, D), BF16),
            vmem((H // 2 * WPITCH, D), U32),
            vmem((H * D, M), BF16),
            vmem((S, M), BF16),
            vmem((M, 3 * M), BF16),
            vmem((2 * NTILE, M // 2, LANES), U32),
            vmem((M, M), BF16),
            vmem((NTILE, DH_B * (H + 1), LANES), F32),
            vmem((M, M), BF16),
            vmem((NTILE, S, LANES), BF16),
            vmem((NTILE, S // 2, LANES), U32),
            vmem((2 * NTILE, HALO + S, LANES), F32),
            vmem((DH_B * (H + 1), LANES), U32),
            vmem((H, S, D), BF16),
            vmem((S, D), BF16),
            vmem((S, D), BF16),
            vmem((BM3, M), BF16),
            vmem((2, BM3, M), BF16),
            vmem((2, BM3, M), BF16),
            pltpu.SemaphoreType.DMA((17,)),
            pltpu.SemaphoreType.DMA((4,)),
        ],
        compiler_params=pltpu.CompilerParams(vmem_limit_bytes=126 * 2**20),
        name="fused_attn",
    )(
        A_x.reshape(S, M), A_c_kv.reshape(S, DC), A_w_q.reshape(M * H, D),
        A_w_uk.reshape(DC * H, D), A_w_uv.reshape(DC * H, D),
        A_w_o.reshape(H * D, M), B_x.reshape(S, M), B_wqkv, B_wo,
    )
    return out.reshape(1, S, 2 * M)
```

```python
import math

import jax
import jax.numpy as jnp
import numpy as np
from jax import lax
import jax.experimental.pallas as pl
import jax.experimental.pallas.tpu as pltpu

S = 2048
M = 1024
DC = 512
H = 32
D = 128
DH_B = 32
WIN, DIL = 8, 2
HALO = 16

LANES = 128
NTILE = M // LANES
BQ = 512
PM = 256
BM3 = 256
WROWS = M + 2 * DC
WPITCH = WROWS + 1
NKV = 8
NQB = 2
R1 = 128
PMA = 128
RA = 256
R2 = 256
FRAC3 = 0.9

LOG2E = math.log2(math.e)
NT = (((1,), (1,)), ((), ()))
BF16 = jnp.bfloat16
F32 = jnp.float32
U32 = jnp.uint32


def _dot(a, b):
    return jnp.dot(a, b, preferred_element_type=F32)


def _dot_nt(a, b):
    return lax.dot_general(a, b, NT, preferred_element_type=F32)


def _recip(x):
    r = pltpu.reciprocal(x, approx=True)
    return r * (2.0 - x * r)


def _ds(start, size, align):
    if not isinstance(start, int):
        start = pl.multiple_of(start, align)
    return pl.ds(start, size)


class _SideWork:
    def __init__(self, step, ndots, *lists):
        keyed = [((i + 0.5) / len(l), j, f)
                 for j, l in enumerate(lists) for i, f in enumerate(l)]
        self.todo = sorted(keyed, key=lambda e: e[:2])
        self.ndots, self.dots, self.last = ndots, 0, None
        self.never = jnp.full((8, LANES), step) < 0

    def dot(self, a, b):
        y = _dot(a, b)
        self.dots += 1
        self.last = y[0:8, 0:LANES]
        while self.todo and self.todo[0][0] * self.ndots <= self.dots:
            self.todo.pop(0)[2]()
        return y

    def pin(self, x):
        last = pltpu.bitcast(self.last, x.dtype)
        return jnp.concatenate([jnp.concatenate(
            [jnp.where(self.never, last, x[r:r + 8, c:c + LANES])
             for c in range(0, x.shape[1], LANES)], axis=1)
            for r in range(0, x.shape[0], 8)], axis=0)


def _low(u):
    return pltpu.bitcast(u << 16, F32)


def _high(u):
    return pltpu.bitcast(u & np.uint32(0xFFFF0000), F32)


def _words(x):
    return pltpu.bitcast(x, U32)


def _bf16(u):
    return pltpu.bitcast(u, BF16)


def _lhs_terms(a11, a12, a21, a22):
    return [a11 + a22, a21 + a22, a11, a22, a11 + a12, a21 - a11, a12 - a22]


def _rhs_terms(b11, b12, b21, b22):
    return [b11 + b22, b11, b12 - b22, b21 - b11, b22, b11 + b12, b21 + b22]


def _word_terms(terms, *blocks):
    lo, hi = [_low(u) for u in blocks], [_high(u) for u in blocks]
    out = []
    for a, b in zip(terms(*lo), terms(*hi)):
        plain = [u for u, l in zip(blocks, lo) if l is a]
        out.append(plain[0] if plain else _words(
            pltpu.pack_elementwise([a, b], packed_dtype=BF16)))
    return out


def _weave(a, b):
    return jnp.concatenate(
        [p[r:r + 16] for r in range(0, a.shape[0], 16) for p in (a, b)], axis=0)


def _combine(product):
    c22 = product(5)
    c12 = product(2)
    c22 = c22 + c12
    m = product(4)
    c12 = c12 + m
    c11 = product(6) - m
    m = product(0)
    c11, c22 = c11 + m, c22 + m
    c21 = product(3)
    c11 = c11 + c21
    m = product(1)
    c21, c22 = c21 + m, c22 - m
    return _weave(c11, c21), _weave(c12, c22)


def _kernel(xa_hbm, c_hbm, wq_hbm, wk_hbm, wv_hbm, woa_hbm, xb_hbm, wqkv_hbm,
            wob_hbm, out_hbm,
            xa_t, c_t, w_pair, woa, wob_t, qb_p, kvb, in_sem, out_sem):
    woa_copy = pltpu.make_async_copy(woa_hbm, woa, in_sem.at[10 + 3 * NKV])

    def phase1(xa, c, w_raw, xb, xb_t, wqkv, wkv_t, wob, wob_tmp, qb, tr_tmp):
        rr, xr = WROWS // NKV, S // NKV

        def xb_copy(i):
            rows = _ds(i * RA, RA, RA)
            return pltpu.make_async_copy(xb_hbm.at[rows], xb.at[rows],
                                         in_sem.at[11 + 3 * NKV + i])

        wq_b = [pltpu.make_async_copy(
            wqkv_hbm.at[:, c0:c0 + 512], wqkv.at[:, c0:c0 + 512],
            in_sem.at[4 + c0 // 512]) for c0 in (0, 512)]

        def wb_copies(i):
            rows = _ds(i * 512, 512, 512)
            return [
                pltpu.make_async_copy(wqkv_hbm.at[rows, M:3 * M],
                                      wqkv.at[rows, M:3 * M], in_sem.at[6 + i]),
                pltpu.make_async_copy(wob_hbm.at[rows], wob.at[rows],
                                      in_sem.at[8 + i])]

        def a_copies(i, w_src):
            rows = _ds(i * xr, xr, xr)
            return [
                pltpu.make_async_copy(w_src, w_raw.at[i], in_sem.at[10 + 3 * i]),
                pltpu.make_async_copy(xa_hbm.at[rows], xa.at[rows],
                                      in_sem.at[11 + 3 * i]),
                pltpu.make_async_copy(c_hbm.at[rows], c.at[rows],
                                      in_sem.at[12 + 3 * i])]

        w_srcs = [w.at[r * H:(r + rr) * H]
                  for w, n in ((wq_hbm, M), (wk_hbm, DC), (wv_hbm, DC))
                  for r in range(0, n, rr)]
        copies = ([wq_b[0]] + [xb_copy(i) for i in range(S // RA)] + [wq_b[1]] +
                  wb_copies(0) + wb_copies(1))
        for i, src in enumerate(w_srcs):
            copies += a_copies(i, src)
        for cp in copies + [woa_copy]:
            cp.start()

        def row_terms(src, dst, row0, pin):
            for t in range(0, src.shape[1], 2 * LANES):
                top = _words(src[_ds(row0, 16, 16), t:t + 2 * LANES])
                bot = _words(src[_ds(row0 + 16, 16, 16), t:t + 2 * LANES])
                terms = _word_terms(_lhs_terms, pin(top[:, :LANES]), top[:, LANES:],
                                    bot[:, :LANES], pin(bot[:, LANES:]))
                for i, u in enumerate(terms):
                    dst[i, _ds(row0 // 4, 8, 8), t // 2:t // 2 + LANES] = u

        def to_d_major(load, store, pin):
            def scatter(t):
                u = _words(load(t))
                ut = jnp.concatenate([pin(u[:8]), u[8:]], axis=0).T
                for j in range(LANES // DH_B):
                    tr_tmp[pl.ds(4 * t + j, DH_B, stride=H + 1), :] = (
                        ut[j * DH_B:(j + 1) * DH_B])

            def gather(t):
                v = jnp.concatenate(
                    [tr_tmp[pl.ds((4 * t + j) * (H + 1), H), :] for j in range(4)],
                    axis=0)
                store(t, v.T)
            return ([lambda t=t: scatter(t) for t in range(NTILE)] +
                    [lambda t=t: gather(t) for t in range(NTILE)])

        def weight_terms(left, right):
            def blocks(u, odd):
                return jnp.concatenate(
                    [u[r:r + 64] for r in range(64 * odd, u.shape[0], 128)], axis=0)
            return _word_terms(_rhs_terms, blocks(left, 0), blocks(right, 0),
                               blocks(left, 1), blocks(right, 1))

        def permute_w(part, r, pin):
            held = []

            def store(t, v):
                held.append(v)
                if t % 2:
                    for i, u in enumerate(weight_terms(*held[-2:])):
                        wkv_t[(part * NTILE + t) // 2, i, _ds(r // 4, 64, 64), :] = u
            c0 = (1 + part) * M
            return to_d_major(
                lambda t: wqkv[_ds(r, 256, 256), c0 + t * LANES:c0 + (t + 1) * LANES],
                store, pin)

        def permute_q(r, pin):
            def store(t, v):
                qb_p[t, _ds(r // 2, LANES, LANES), :] = v
            return to_d_major(lambda t: qb[t, _ds(r, 256, 256), :], store, pin)

        def project_pair(side, weight, store):
            for r in range(0, S // 2, R1):
                ys = _combine(lambda i: side.dot(
                    _bf16(xb_t[i, r // 2:(r + R1) // 2, :]), _bf16(weight(i))))
                for j, y in enumerate(ys):
                    store(j, 2 * r, y)

        ndots = 7 * S // (2 * R1)
        for t in range(2 * NTILE):
            kvb[t, 0:HALO, :] = jnp.zeros((HALO, LANES), F32)
        wq_b[0].wait()

        def q_step_a(i, carry):
            xb_copy(i).wait()
            side = _SideWork(
                i, 4 * RA // PMA - 1,
                [lambda r=r: row_terms(xb, xb_t, i * RA + r, side.pin)
                 for r in range(0, RA, 32)])
            for r in range(0, RA, PMA):
                rows = _ds(i * RA + r, PMA, PMA)
                for t in range(4):
                    qb[t, rows, :] = side.dot(
                        xb[rows, :], wqkv[:, t * LANES:(t + 1) * LANES]).astype(BF16)
            return carry

        lax.fori_loop(0, S // RA, q_step_a, 0)
        wq_b[1].wait()

        def q_step_b(i, carry):
            for cp in wb_copies(i):
                cp.wait()

            def scatter_wob(h):
                y = side.pin(wob[_ds(h * DH_B, DH_B, DH_B), :].astype(F32))
                for t in range(NTILE):
                    wob_tmp[t, pl.ds(h, DH_B, stride=H + 1), :] = (
                        y[:, t * LANES:(t + 1) * LANES])

            def store(j, r, y):
                qb[4 + 2 * i + j, r:r + 2 * R1, :] = y.astype(BF16)

            perm = []
            for part in range(2):
                for r in (0, 256):
                    perm += permute_w(part, i * 512 + r, lambda x: side.pin(x))
            side = _SideWork(
                i, ndots - 4, perm,
                [lambda j=j: scatter_wob(i * 16 + j) for j in range(16)])
            w = _words(wqkv[:, _ds(512 + i * 256, 256, 256)])
            w = weight_terms(w[:, :LANES], w[:, LANES:])
            project_pair(side, lambda t: w[t], store)
            return carry

        lax.fori_loop(0, NQB, q_step_b, 0)

        def kv_step(i, carry):
            for cp in a_copies(i, w_srcs[0]):
                cp.wait()

            def store(j, r, y):
                kvb[2 * i + j, HALO + r:HALO + r + 2 * R1, :] = y

            def split_pairs(r):
                v = side.pin(_words(w_raw[i, r * H:(r + 8) * H, :]))
                for m in range(8):
                    w_pair[pl.ds(i * rr + r + m, H // 2, stride=WPITCH), :] = (
                        v[m * H // 2:(m + 1) * H // 2])

            def wob_terms(d, c0):
                b = [side.pin(wob_tmp[t, pl.ds(e * (H + 1), H), :])
                     for e in (d, d + (DH_B // 2)) for t in (c0, c0 + NTILE // 2)]
                for j, y in enumerate(_rhs_terms(*b)):
                    wob_t[j, _ds(d * H, H, H), c0 * LANES:(c0 + 1) * LANES] = y.astype(BF16)

            nd = DH_B // 2 // NKV
            side = _SideWork(
                i, ndots - 4,
                [lambda r=r: split_pairs(r) for r in range(0, rr, 8)],
                permute_q(i * xr, lambda x: side.pin(x)),
                [lambda j=j, c0=c0: wob_terms(i * nd + j, c0)
                 for j in range(nd) for c0 in range(NTILE // 2)],
                [lambda r=r: row_terms(xa, xa_t, i * xr + r, side.pin)
                 for r in range(0, xr, 32)],
                [lambda r=r: row_terms(c, c_t, i * xr + r, side.pin)
                 for r in range(0, xr, 32)])
            project_pair(side, lambda t: wkv_t[i, t], store)
            return carry

        lax.fori_loop(0, NKV, kv_step, 0)

    pl.run_scoped(
        phase1,
        pltpu.VMEM((S, M), BF16),
        pltpu.VMEM((S, DC), BF16),
        pltpu.VMEM((NKV, WROWS // NKV * H, D), BF16),
        pltpu.VMEM((S, M), BF16),
        pltpu.VMEM((7, S // 4, M // 2), U32),
        pltpu.VMEM((M, 3 * M), BF16),
        pltpu.VMEM((NTILE, 7, M // 4, LANES), U32),
        pltpu.VMEM((M, M), BF16),
        pltpu.VMEM((NTILE, DH_B * (H + 1), LANES), F32),
        pltpu.VMEM((NTILE, S, LANES), BF16),
        pltpu.VMEM((DH_B * (H + 1), LANES), U32),
    )
    woa_copy.wait()

    def phase23(ctx_t, woa_t, ks, vs, att_t, oa_buf, ob_buf):
        q_scale = D ** -0.5 * LOG2E
        nt = BQ // LANES
        strips = [slice(a * LANES, (a + 1) * LANES) for a in range(nt)]

        def attend(j, r0, q, causal):
            s = [[] for _ in range(nt)]
            if r0:
                past = _dot_nt(q.astype(BF16), ks[j, 0:r0, :])
                for a in range(nt):
                    s[a].append(past[strips[a]])
            for a in range(nt):
                near = _dot_nt(q[strips[a]].astype(BF16),
                               ks[j, r0:r0 + (a + 1) * LANES, :])
                if a:
                    s[a].append(near[:, :a * LANES])
                s[a].append(jnp.where(causal, near[:, a * LANES:], -1e30))
            p, inv = [], []
            for a in range(nt):
                sa = jnp.concatenate(s[a], axis=1)
                pa = jnp.exp2(sa - jnp.max(sa, axis=1, keepdims=True))
                inv.append(_recip(jnp.sum(pa, axis=1, keepdims=True)))
                p.append(pa)
            if r0:
                p_past = jnp.concatenate([pa[:, :r0] for pa in p], axis=0)
                o_past = _dot(p_past.astype(BF16), vs[j, 0:r0, :])
            out = []
            for a in range(nt):
                o = _dot(p[a][:, r0:].astype(BF16), vs[j, r0:r0 + (a + 1) * LANES, :])
                if r0:
                    o = o + o_past[strips[a]]
                out.append(o * inv[a])
            return out

        def pair_step(pair, carry):
            def weight_terms(row0, n):
                top, bot = [jnp.concatenate(
                    [w_pair[pl.ds(pair * WPITCH + row0 + r, LANES), :]
                     for r in range(odd * LANES, 2 * n, 2 * LANES)], axis=0)
                    for odd in (0, 1)]
                return _rhs_terms(_low(top), _high(top), _low(bot), _high(bot))

            row = lax.broadcasted_iota(jnp.int32, (LANES, LANES), 0)
            col = lax.broadcasted_iota(jnp.int32, (LANES, LANES), 1)
            causal = col <= row
            wkv = [jnp.concatenate([a, b], axis=1).astype(BF16) for a, b in zip(
                weight_terms(M, DC // 2), weight_terms(M + DC, DC // 2))]
            for r in range(0, S // 2, R2):
                kv = _combine(lambda i: _dot(
                    _bf16(c_t[i, r // 2:(r + R2) // 2, :]), wkv[i]))
                for j in range(2):
                    ks[j, 2 * r:2 * (r + R2), :] = kv[j][:, :D].astype(BF16)
                    vs[j, 2 * r:2 * (r + R2), :] = kv[j][:, D:].astype(BF16)
            for r in range(0, D, 16):
                top = _words(woa[_ds(pair * 2 * D + r, 16, 16), :])
                bot = _words(woa[_ds(pair * 2 * D + D + r, 16, 16), :])
                half = M // 2
                for i, u in enumerate(_word_terms(
                        _rhs_terms, top[:, :half], top[:, half:],
                        bot[:, :half], bot[:, half:])):
                    woa_t[i, _ds((pair * D + r) // 2, 8, 8), :] = u
            wq = [a.astype(BF16) for a in weight_terms(0, M // 2)]
            for r0 in range(S - BQ, -1, -BQ):
                q = _combine(lambda i: _dot(
                    _bf16(xa_t[i, r0 // 4:(r0 + BQ) // 4, :]), wq[i]))
                o = [attend(j, r0, q[j] * q_scale, causal) for j in range(2)]
                for a in range(nt):
                    for r in range(0, LANES, 32):
                        terms = _lhs_terms(o[0][a][r:r + 16], o[1][a][r:r + 16],
                                           o[0][a][r + 16:r + 32], o[1][a][r + 16:r + 32])
                        dst = (r0 + a * LANES + r) // 2
                        for i, y in enumerate(terms):
                            ctx_t[i, pair, dst:dst + 16, :] = y.astype(BF16)
            return carry

        lax.fori_loop(0, H // 2, pair_step, 0)

        nblk = S // BM3
        b_scale = DH_B ** -0.5 * LOG2E

        def out_copies(i, slot):
            rows = _ds(i * BM3, BM3, BM3)
            return (
                pltpu.make_async_copy(oa_buf.at[slot], out_hbm.at[rows, 0:M],
                                      out_sem.at[2 * slot]),
                pltpu.make_async_copy(ob_buf.at[slot], out_hbm.at[rows, M:2 * M],
                                      out_sem.at[2 * slot + 1]),
            )

        def window_attention(r0, a, prev):
            n = 16
            pos = r0 + a + lax.broadcasted_iota(jnp.int32, (n, LANES), 0)
            q = [_bf16(qb_p[t, _ds((r0 + a) // 2, n // 2, 8), :]).astype(F32)
                 for t in range(NTILE)]
            if prev:
                q[0] = jnp.where(pos < 0, prev[-1][-1], q[0])
            src = [pl.ds(r0 + HALO + a - DIL * w, n) for w in range(WIN)]
            logits = []
            for w in range(WIN):
                l = q[0] * kvb[0, src[w], :]
                for t in range(1, NTILE):
                    l = l + q[t] * kvb[t, src[w], :]
                l = l + pltpu.roll(l, 2 * H, 1)
                l = (l + pltpu.roll(l, H, 1)) * b_scale
                if DIL * w > a:
                    l = jnp.where(pos >= DIL * w, l, -1e30)
                logits.append(l)
            m = logits[0]
            for l in logits[1:]:
                m = jnp.maximum(m, l)
            e = [jnp.exp2(l - m) for l in logits]
            total = e[0]
            for x in e[1:]:
                total = total + x
            inv = _recip(total)
            e = [x * inv for x in e]
            o = []
            for t in range(NTILE):
                acc = e[0] * kvb[NTILE + t, src[0], :]
                for w in range(1, WIN):
                    acc = acc + e[w] * kvb[NTILE + t, src[w], :]
                o.append(acc)
            prev.append(o)
            if a % 32:
                blocks = [jnp.concatenate(x, axis=1)
                          for o in prev[-2:] for x in (o[:NTILE // 2], o[NTILE // 2:])]
                for i, y in enumerate(_lhs_terms(*blocks)):
                    att_t[i, a // 32 * 16:a // 32 * 16 + 16, :] = y.astype(BF16)

        def out_step(i, carry):
            slot = i % 2
            r0 = pl.multiple_of(i * BM3, BM3)

            @pl.when(i >= 2)
            def _():
                for cp in out_copies(i - 2, slot):
                    cp.wait()

            def store(buf, n, ys):
                for j, y in enumerate(ys):
                    c0 = j * M // 2 + n
                    buf[slot, :, c0:c0 + LANES] = y.astype(BF16)

            prev = []
            side = _SideWork(
                i, int(FRAC3 * 7 * M // (2 * LANES)),
                [lambda a=a: window_attention(r0, a, prev) for a in range(0, BM3, 16)])
            rows = _ds(r0 // 2, BM3 // 2, BM3 // 2)
            for n in range(0, M // 2, LANES):
                store(oa_buf, n, _combine(lambda t: side.dot(
                    jnp.concatenate([ctx_t[t, p, rows, :] for p in range(H // 2)], axis=1),
                    _bf16(woa_t[t, :, n:n + LANES]))))
            for n in range(0, M // 2, LANES):
                store(ob_buf, n, _combine(
                    lambda t: _dot(att_t[t], wob_t[t, :, n:n + LANES])))
            for cp in out_copies(i, slot):
                cp.start()
            return carry

        lax.fori_loop(0, nblk, out_step, 0)
        for i in (nblk - 2, nblk - 1):
            for cp in out_copies(i, i % 2):
                cp.wait()

    pl.run_scoped(
        phase23,
        pltpu.VMEM((7, H // 2, S // 2, D), BF16),
        pltpu.VMEM((7, H * D // 4, M // 2), U32),
        pltpu.VMEM((2, S, D), BF16),
        pltpu.VMEM((2, S, D), BF16),
        pltpu.VMEM((7, BM3 // 2, M // 2), BF16),
        pltpu.VMEM((2, BM3, M), BF16),
        pltpu.VMEM((2, BM3, M), BF16),
    )


@jax.jit
def pallas_concat_heads__compressed_kv_cla__sliding_local_dilated__prompt_kernel(
    A_x: jax.Array,
    A_c_kv: jax.Array,
    A_w_q: jax.Array,
    A_w_uk: jax.Array,
    A_w_uv: jax.Array,
    A_w_o: jax.Array,
    B_x: jax.Array,
    B_wqkv: jax.Array,
    B_wo: jax.Array,
):
    vmem = pltpu.VMEM
    out = pl.pallas_call(
        _kernel,
        out_shape=jax.ShapeDtypeStruct((S, 2 * M), BF16),
        in_specs=[pl.BlockSpec(memory_space=pl.ANY)] * 9,
        out_specs=pl.BlockSpec(memory_space=pl.ANY),
        scratch_shapes=[
            vmem((7, S // 4, M // 2), U32),
            vmem((7, S // 4, DC // 2), U32),
            vmem((H // 2 * WPITCH, D), U32),
            vmem((H * D, M), BF16),
            vmem((7, M // 2, M // 2), BF16),
            vmem((NTILE, S // 2, LANES), U32),
            vmem((2 * NTILE, HALO + S, LANES), F32),
            pltpu.SemaphoreType.DMA((11 + 3 * NKV + S // RA,)),
            pltpu.SemaphoreType.DMA((4,)),
        ],
        compiler_params=pltpu.CompilerParams(vmem_limit_bytes=126 * 2**20),
        name="fused_attn",
    )(
        A_x.reshape(S, M), A_c_kv.reshape(S, DC), A_w_q.reshape(M * H, D),
        A_w_uk.reshape(DC * H, D), A_w_uv.reshape(DC * H, D),
        A_w_o.reshape(H * D, M), B_x.reshape(S, M), B_wqkv, B_wo,
    )
    return out.reshape(1, S, 2 * M)
```

```python
import math

import jax
import jax.numpy as jnp
import numpy as np
from jax import lax
import jax.experimental.pallas as pl
import jax.experimental.pallas.tpu as pltpu

S = 2048
M = 1024
DC = 512
H = 32
D = 128
DH_B = 32
WIN, DIL = 8, 2
HALO = 16

LANES = 128
NTILE = M // LANES
BQ = 512
PM = 256
BM3 = 256
WROWS = M + 2 * DC
WPITCH = WROWS + 1
NKV = 8
NQB = 2
R1 = 128
PMA = 128
RA = 256
KS3 = 4
AFTER = True
ORDER = '01236789abcdef45'
AHEAD = 1
CHAIN = True
R2 = 256
FRAC3 = 0.9

LOG2E = math.log2(math.e)
NT = (((1,), (1,)), ((), ()))
BF16 = jnp.bfloat16
F32 = jnp.float32
U32 = jnp.uint32


def _dot(a, b):
    return jnp.dot(a, b, preferred_element_type=F32)


def _dot_nt(a, b):
    return lax.dot_general(a, b, NT, preferred_element_type=F32)


def _recip(x):
    r = pltpu.reciprocal(x, approx=True)
    return r * (2.0 - x * r)


def _ds(start, size, align):
    if not isinstance(start, int):
        start = pl.multiple_of(start, align)
    return pl.ds(start, size)


class _SideWork:
    def __init__(self, step, ndots, *lists):
        keyed = [((i + 0.5) / len(l), j, f)
                 for j, l in enumerate(lists) for i, f in enumerate(l)]
        self.todo = sorted(keyed, key=lambda e: e[:2])
        self.ndots, self.dots, self.last, self.done = ndots, 0, None, None
        self.never = jnp.full((8, LANES), step) < 0

    def dot(self, a, b):
        y = _dot(a, b)
        self.dots += 1
        self.last = y[0:8, 0:LANES]
        while self.todo and self.todo[0][0] * self.ndots <= self.dots:
            self.done = self.todo.pop(0)[2]()
        return y

    def after(self, x):
        if self.done is None:
            return x
        done, self.done = pltpu.bitcast(self.done[0:8, 0:LANES], x.dtype), None
        return jnp.concatenate([jnp.where(self.never, done, x[:8]), x[8:]], axis=0)

    def pin(self, x):
        last = pltpu.bitcast(self.last, x.dtype)
        return jnp.concatenate([jnp.concatenate(
            [jnp.where(self.never, last, x[r:r + 8, c:c + LANES])
             for c in range(0, x.shape[1], LANES)], axis=1)
            for r in range(0, x.shape[0], 8)], axis=0)


def _low(u):
    return pltpu.bitcast(u << 16, F32)


def _high(u):
    return pltpu.bitcast(u & np.uint32(0xFFFF0000), F32)


def _words(x):
    return pltpu.bitcast(x, U32)


def _bf16(u):
    return pltpu.bitcast(u, BF16)


def _lhs_terms(a11, a12, a21, a22):
    return [a11 + a22, a21 + a22, a11, a22, a11 + a12, a21 - a11, a12 - a22]


def _rhs_terms(b11, b12, b21, b22):
    return [b11 + b22, b11, b12 - b22, b21 - b11, b22, b11 + b12, b21 + b22]


def _word_terms(terms, *blocks):
    lo, hi = [_low(u) for u in blocks], [_high(u) for u in blocks]
    out = []
    for a, b in zip(terms(*lo), terms(*hi)):
        plain = [u for u, l in zip(blocks, lo) if l is a]
        out.append(plain[0] if plain else _words(
            pltpu.pack_elementwise([a, b], packed_dtype=BF16)))
    return out


def _weave(a, b):
    return jnp.concatenate(
        [p[r:r + 16] for r in range(0, a.shape[0], 16) for p in (a, b)], axis=0)


def _combine(product):
    c22 = product(5)
    c12 = product(2)
    c22 = c22 + c12
    m = product(4)
    c12 = c12 + m
    c11 = product(6) - m
    m = product(0)
    c11, c22 = c11 + m, c22 + m
    c21 = product(3)
    c11 = c11 + c21
    m = product(1)
    c21, c22 = c21 + m, c22 - m
    return _weave(c11, c21), _weave(c12, c22)


def _kernel(xa_hbm, c_hbm, wq_hbm, wk_hbm, wv_hbm, woa_hbm, xb_hbm, wqkv_hbm,
            wob_hbm, out_hbm,
            xa_t, c_t, w_pair, woa, wob_t, qb_p, kvb, in_sem, out_sem):
    woa_copy = pltpu.make_async_copy(woa_hbm, woa, in_sem.at[10 + 3 * NKV])

    def phase1(xa, c, w_raw, xb, xb_t, wqkv, wkv_t, wob, wob_tmp, qb, tr_tmp):
        rr, xr = WROWS // NKV, S // NKV

        def xb_copy(i):
            rows = _ds(i * RA, RA, RA)
            return pltpu.make_async_copy(xb_hbm.at[rows], xb.at[rows],
                                         in_sem.at[11 + 3 * NKV + i])

        wq_b = [pltpu.make_async_copy(
            wqkv_hbm.at[:, c0:c0 + 512], wqkv.at[:, c0:c0 + 512],
            in_sem.at[4 + c0 // 512]) for c0 in (0, 512)]

        def wb_copies(i):
            rows = _ds(i * 512, 512, 512)
            return [
                pltpu.make_async_copy(wqkv_hbm.at[rows, M:3 * M],
                                      wqkv.at[rows, M:3 * M], in_sem.at[6 + i]),
                pltpu.make_async_copy(wob_hbm.at[rows], wob.at[rows],
                                      in_sem.at[8 + i])]

        def a_copies(i, w_src):
            rows = _ds(i * xr, xr, xr)
            return [
                pltpu.make_async_copy(w_src, w_raw.at[i], in_sem.at[10 + 3 * i]),
                pltpu.make_async_copy(xa_hbm.at[rows], xa.at[rows],
                                      in_sem.at[11 + 3 * i]),
                pltpu.make_async_copy(c_hbm.at[rows], c.at[rows],
                                      in_sem.at[12 + 3 * i])]

        w_srcs = [w.at[r * H:(r + rr) * H]
                  for w, n in ((wq_hbm, M), (wk_hbm, DC), (wv_hbm, DC))
                  for r in range(0, n, rr)]
        copies = ([wq_b[0]] + [xb_copy(i) for i in range(S // RA)] + [wq_b[1]] +
                  wb_copies(0) + wb_copies(1))
        for i, src in enumerate(w_srcs):
            copies += a_copies(i, src)
        for cp in copies + [woa_copy]:
            cp.start()

        def row_terms(src, dst, row0, pin):
            for t in range(0, src.shape[1], 2 * LANES):
                top = _words(src[_ds(row0, 16, 16), t:t + 2 * LANES])
                bot = _words(src[_ds(row0 + 16, 16, 16), t:t + 2 * LANES])
                terms = _word_terms(_lhs_terms, pin(top[:, :LANES]), top[:, LANES:],
                                    bot[:, :LANES], pin(bot[:, LANES:]))
                for i, u in enumerate(terms):
                    dst[i, _ds(row0 // 4, 8, 8), t // 2:t // 2 + LANES] = u

        def to_d_major(load, store, pin):
            def scatter(t):
                u = _words(load(t))
                ut = jnp.concatenate([pin(u[:8]), u[8:]], axis=0).T
                for j in range(LANES // DH_B):
                    tr_tmp[pl.ds(4 * t + j, DH_B, stride=H + 1), :] = (
                        ut[j * DH_B:(j + 1) * DH_B])

            def gather(t):
                v = jnp.concatenate(
                    [tr_tmp[pl.ds((4 * t + j) * (H + 1), H), :] for j in range(4)],
                    axis=0)
                store(t, v.T)
            return ([lambda t=t: scatter(t) for t in range(NTILE)] +
                    [lambda t=t: gather(t) for t in range(NTILE)])

        def weight_terms(left, right):
            def blocks(u, odd):
                return jnp.concatenate(
                    [u[r:r + 64] for r in range(64 * odd, u.shape[0], 128)], axis=0)
            return _word_terms(_rhs_terms, blocks(left, 0), blocks(right, 0),
                               blocks(left, 1), blocks(right, 1))

        def permute_w(part, r, pin):
            held = []

            def store(t, v):
                held.append(v)
                if t % 2:
                    for i, u in enumerate(weight_terms(*held[-2:])):
                        wkv_t[(part * NTILE + t) // 2, i, _ds(r // 4, 64, 64), :] = u
            c0 = (1 + part) * M
            return to_d_major(
                lambda t: wqkv[_ds(r, 256, 256), c0 + t * LANES:c0 + (t + 1) * LANES],
                store, pin)

        def permute_q(r, pin):
            def store(t, v):
                qb_p[t, _ds(r // 2, LANES, LANES), :] = v
            return to_d_major(lambda t: qb[t, _ds(r, 256, 256), :], store, pin)

        def project_pair(side, weight, store):
            for r in range(0, S // 2, R1):
                ys = _combine(lambda i: side.dot(
                    _bf16(xb_t[i, r // 2:(r + R1) // 2, :]), _bf16(weight(i))))
                for j, y in enumerate(ys):
                    store(j, 2 * r, y)

        ndots = 7 * S // (2 * R1)
        for t in range(2 * NTILE):
            kvb[t, 0:HALO, :] = jnp.zeros((HALO, LANES), F32)
        wq_b[0].wait()

        def q_step_a(i, carry):
            xb_copy(i).wait()
            side = _SideWork(
                i, 4 * RA // PMA - 1,
                [lambda r=r: row_terms(xb, xb_t, i * RA + r, side.pin)
                 for r in range(0, RA, 32)])
            for r in range(0, RA, PMA):
                rows = _ds(i * RA + r, PMA, PMA)
                for t in range(4):
                    qb[t, rows, :] = side.dot(
                        xb[rows, :], wqkv[:, t * LANES:(t + 1) * LANES]).astype(BF16)
            return carry

        lax.fori_loop(0, S // RA, q_step_a, 0)
        wq_b[1].wait()

        def q_step_b(i, carry):
            for cp in wb_copies(i):
                cp.wait()

            def scatter_wob(h):
                y = side.pin(wob[_ds(h * DH_B, DH_B, DH_B), :].astype(F32))
                for t in range(NTILE):
                    wob_tmp[t, pl.ds(h, DH_B, stride=H + 1), :] = (
                        y[:, t * LANES:(t + 1) * LANES])

            def store(j, r, y):
                qb[4 + 2 * i + j, r:r + 2 * R1, :] = y.astype(BF16)

            perm = []
            for part in range(2):
                for r in (0, 256):
                    perm += permute_w(part, i * 512 + r, lambda x: side.pin(x))
            side = _SideWork(
                i, ndots - 4, perm,
                [lambda j=j: scatter_wob(i * 16 + j) for j in range(16)])
            w = _words(wqkv[:, _ds(512 + i * 256, 256, 256)])
            w = weight_terms(w[:, :LANES], w[:, LANES:])
            project_pair(side, lambda t: w[t], store)
            return carry

        lax.fori_loop(0, NQB, q_step_b, 0)

        def kv_step(i, carry):
            for cp in a_copies(i, w_srcs[0]):
                cp.wait()

            def store(j, r, y):
                kvb[2 * i + j, HALO + r:HALO + r + 2 * R1, :] = y

            def split_pairs(r):
                v = side.pin(_words(w_raw[i, r * H:(r + 8) * H, :]))
                for m in range(8):
                    w_pair[pl.ds(i * rr + r + m, H // 2, stride=WPITCH), :] = (
                        v[m * H // 2:(m + 1) * H // 2])

            def wob_terms(d, c0):
                b = [side.pin(wob_tmp[t, pl.ds(e * (H + 1), H), :])
                     for e in (d, d + (DH_B // 2)) for t in (c0, c0 + NTILE // 2)]
                for j, y in enumerate(_rhs_terms(*b)):
                    wob_t[j, _ds(d * H, H, H), c0 * LANES:(c0 + 1) * LANES] = y.astype(BF16)

            nd = DH_B // 2 // NKV
            side = _SideWork(
                i, ndots - 4,
                [lambda r=r: split_pairs(r) for r in range(0, rr, 8)],
                permute_q(i * xr, lambda x: side.pin(x)),
                [lambda j=j, c0=c0: wob_terms(i * nd + j, c0)
                 for j in range(nd) for c0 in range(NTILE // 2)],
                [lambda r=r: row_terms(xa, xa_t, i * xr + r, side.pin)
                 for r in range(0, xr, 32)],
                [lambda r=r: row_terms(c, c_t, i * xr + r, side.pin)
                 for r in range(0, xr, 32)])
            project_pair(side, lambda t: wkv_t[i, t], store)
            return carry

        lax.fori_loop(0, NKV, kv_step, 0)

    pl.run_scoped(
        phase1,
        pltpu.VMEM((S, M), BF16),
        pltpu.VMEM((S, DC), BF16),
        pltpu.VMEM((NKV, WROWS // NKV * H, D), BF16),
        pltpu.VMEM((S, M), BF16),
        pltpu.VMEM((7, S // 4, M // 2), U32),
        pltpu.VMEM((M, 3 * M), BF16),
        pltpu.VMEM((NTILE, 7, M // 4, LANES), U32),
        pltpu.VMEM((M, M), BF16),
        pltpu.VMEM((NTILE, DH_B * (H + 1), LANES), F32),
        pltpu.VMEM((NTILE, S, LANES), BF16),
        pltpu.VMEM((DH_B * (H + 1), LANES), U32),
    )
    woa_copy.wait()

    def phase23(ctx_t, woa_t, ks, vs, att_t, oa_buf, ob_buf):
        q_scale = D ** -0.5 * LOG2E

        def pair_step(pair, carry):
            def weight_terms(row0, n):
                top, bot = [jnp.concatenate(
                    [w_pair[pl.ds(pair * WPITCH + row0 + r, LANES), :]
                     for r in range(odd * LANES, n, 2 * LANES)], axis=0)
                    for odd in (0, 1)]
                return _rhs_terms(_low(top), _high(top), _low(bot), _high(bot))

            def out_weight_terms(r, t):
                top, bot = [_words(woa[_ds(pair * 2 * D + j * D + r, 16, 16),
                                       t * LANES:(t + 2) * LANES]) for j in range(2)]
                for i, u in enumerate(_word_terms(
                        _rhs_terms, side.pin(top[:, :LANES]), top[:, LANES:],
                        bot[:, :LANES], side.pin(bot[:, LANES:]))):
                    woa_t[t // 2, i, _ds((pair * D + r) // 2, 8, 8), :] = u

            side = _SideWork(
                pair, 7 * NTILE,
                [lambda r=r, t=t: out_weight_terms(r, t)
                 for r in range(0, D, 16) for t in range(0, NTILE, 2)])
            row = lax.broadcasted_iota(jnp.int32, (LANES, LANES), 0)
            col = lax.broadcasted_iota(jnp.int32, (LANES, LANES), 1)
            causal = col <= row
            never = jnp.full((LANES, LANES), pair) < 0
            wkv = [jnp.concatenate([a, b], axis=1).astype(BF16) for a, b in zip(
                weight_terms(M, DC), weight_terms(M + DC, DC))]
            wq = [a.astype(BF16) for a in weight_terms(0, M)]
            q, ctx = {}, {}

            def project_kv(g):
                kv = _combine(lambda i: side.dot(
                    _bf16(c_t[i, g * 64:(g + 1) * 64, :]), wkv[i]))
                for j in range(2):
                    ks[j, g * 256:(g + 1) * 256, :] = kv[j][:, :D].astype(BF16)
                    vs[j, g * 256:(g + 1) * 256, :] = kv[j][:, D:].astype(BF16)

            def project_q(g):
                ys = _combine(lambda i: _dot(
                    _bf16(xa_t[i, g * 64:(g + 1) * 64, :]), wq[i]))
                for j, y in enumerate(ys):
                    q[j, 2 * g] = y[:LANES] * q_scale
                    q[j, 2 * g + 1] = y[LANES:] * q_scale

            def scores(j, a):
                s = _dot_nt(q[j, a].astype(BF16), ks[j, 0:(a + 1) * LANES, :])
                s = [s[:, t * LANES:(t + 1) * LANES] for t in range(a + 1)]
                s[a] = jnp.where(causal, s[a], -1e30)
                return s

            def attend(j, a, s):
                m = s[0]
                for x in s[1:]:
                    m = jnp.maximum(m, x)
                m = jnp.max(m, axis=1, keepdims=True)
                p = [jnp.exp2(x - m) for x in s]
                total = p[0]
                for x in p[1:]:
                    total = total + x
                if a:
                    p[a] = jnp.where(never, total, p[a])
                o = _dot(jnp.concatenate(p, axis=1).astype(BF16),
                         vs[j, 0:(a + 1) * LANES, :])
                ctx[j, a] = o * _recip(jnp.sum(total, axis=1, keepdims=True))
                if j:
                    for r in range(0, LANES, 32):
                        terms = _lhs_terms(
                            ctx[0, a][r:r + 16], ctx[1, a][r:r + 16],
                            ctx[0, a][r + 16:r + 32], ctx[1, a][r + 16:r + 32])
                        dst = (a * LANES + r) // 2
                        for i, y in enumerate(terms):
                            ctx_t[i, pair, dst:dst + 16, :] = y.astype(BF16)

            strips = [(j, int(a, 16)) for a in ORDER for j in range(2)]
            kv_done, waiting = 0, None
            for n, (j, a) in enumerate(strips):
                while kv_done < min(NTILE, max(n + 1, a // 2 + 1)):
                    project_kv(kv_done)
                    kv_done += 1
                for key in strips[n:n + 1 + AHEAD]:
                    if key not in q:
                        project_q(key[1] // 2)
                s = scores(j, a)
                if waiting:
                    attend(*waiting)
                waiting = (j, a, s)
            attend(*waiting)
            return carry

        lax.fori_loop(0, H // 2, pair_step, 0)

        nblk = S // BM3
        b_scale = DH_B ** -0.5 * LOG2E

        def out_copies(i, slot):
            return (
                pltpu.make_async_copy(
                    oa_buf.at[slot],
                    out_hbm.at[_ds(i // 2 * 2 * BM3, 2 * BM3, BM3),
                               _ds(slot * (M // 2), M // 2, M // 2)],
                    out_sem.at[2 * slot]),
                pltpu.make_async_copy(
                    ob_buf.at[slot], out_hbm.at[_ds(i * BM3, BM3, BM3), M:2 * M],
                    out_sem.at[2 * slot + 1]),
            )

        def window_attention(r0, a, prev):
            n = 16
            pos = r0 + a + lax.broadcasted_iota(jnp.int32, (n, LANES), 0)
            q = [_bf16(qb_p[t, _ds((r0 + a) // 2, n // 2, 8), :]).astype(F32)
                 for t in range(NTILE)]
            if prev and CHAIN:
                q[0] = jnp.where(pos < 0, prev[-1][-1], q[0])
            src = [pl.ds(r0 + HALO + a - DIL * w, n) for w in range(WIN)]
            logits = []
            for w in range(WIN):
                l = q[0] * kvb[0, src[w], :]
                for t in range(1, NTILE):
                    l = l + q[t] * kvb[t, src[w], :]
                l = l + pltpu.roll(l, 2 * H, 1)
                l = (l + pltpu.roll(l, H, 1)) * b_scale
                if DIL * w > a:
                    l = jnp.where(pos >= DIL * w, l, -1e30)
                logits.append(l)
            m = logits[0]
            for l in logits[1:]:
                m = jnp.maximum(m, l)
            e = [jnp.exp2(l - m) for l in logits]
            total = e[0]
            for x in e[1:]:
                total = total + x
            inv = _recip(total)
            e = [x * inv for x in e]
            o = []
            for t in range(NTILE):
                acc = e[0] * kvb[NTILE + t, src[0], :]
                for w in range(1, WIN):
                    acc = acc + e[w] * kvb[NTILE + t, src[w], :]
                o.append(acc)
            prev.append(o)
            if a % 32:
                blocks = [jnp.concatenate(x, axis=1)
                          for o in prev[-2:] for x in (o[:NTILE // 2], o[NTILE // 2:])]
                for i, y in enumerate(_lhs_terms(*blocks)):
                    att_t[i, a // 32 * 16:a // 32 * 16 + 16, :] = y.astype(BF16)
            return o[-1] if AFTER else None

        def out_step(i, carry):
            slot = i % 2
            r0 = pl.multiple_of(i * BM3, BM3)

            @pl.when(i >= 2)
            def _():
                for cp in out_copies(i - 2, slot):
                    cp.wait()

            def store(buf, n, ys):
                for j, y in enumerate(ys):
                    c0 = j * M // 2 + n
                    buf[slot, :, c0:c0 + LANES] = y.astype(BF16)

            prev = []
            side = _SideWork(
                i, int(FRAC3 * 7 * 2 * KS3),
                [lambda a=a: window_attention(r0, a, prev) for a in range(0, BM3, 16)])
            rows = _ds(i // 2 * BM3, BM3, BM3)

            def product(n, t):
                y = None
                np_ = H // 2 // KS3
                for k in range(0, H // 2, np_):
                    part = side.dot(
                        jnp.concatenate(
                            [ctx_t[t, p, rows, :] for p in range(k, k + np_)], axis=1),
                        _bf16(side.after(woa_t[2 * slot + n, t, k * D // 2:(k + np_) * D // 2, :])))
                    y = part if y is None else y + part
                return y

            for n in range(2):
                for j, y in enumerate(_combine(lambda t: product(n, t))):
                    oa_buf[slot, :, (2 * n + j) * LANES:(2 * n + j + 1) * LANES] = (
                        y.astype(BF16))
            for n in range(0, M // 2, LANES):
                store(ob_buf, n, _combine(
                    lambda t: _dot(att_t[t], wob_t[t, :, n:n + LANES])))
            for cp in out_copies(i, slot):
                cp.start()
            return carry

        lax.fori_loop(0, nblk, out_step, 0)
        for i in (nblk - 2, nblk - 1):
            for cp in out_copies(i, i % 2):
                cp.wait()

    pl.run_scoped(
        phase23,
        pltpu.VMEM((7, H // 2, S // 2, D), BF16),
        pltpu.VMEM((NTILE // 2, 7, H * D // 4, LANES), U32),
        pltpu.VMEM((2, S, D), BF16),
        pltpu.VMEM((2, S, D), BF16),
        pltpu.VMEM((7, BM3 // 2, M // 2), BF16),
        pltpu.VMEM((2, 2 * BM3, M // 2), BF16),
        pltpu.VMEM((2, BM3, M), BF16),
    )


@jax.jit
def pallas_concat_heads__compressed_kv_cla__sliding_local_dilated__prompt_kernel(
    A_x: jax.Array,
    A_c_kv: jax.Array,
    A_w_q: jax.Array,
    A_w_uk: jax.Array,
    A_w_uv: jax.Array,
    A_w_o: jax.Array,
    B_x: jax.Array,
    B_wqkv: jax.Array,
    B_wo: jax.Array,
):
    vmem = pltpu.VMEM
    out = pl.pallas_call(
        _kernel,
        out_shape=jax.ShapeDtypeStruct((S, 2 * M), BF16),
        in_specs=[pl.BlockSpec(memory_space=pl.ANY)] * 9,
        out_specs=pl.BlockSpec(memory_space=pl.ANY),
        scratch_shapes=[
            vmem((7, S // 4, M // 2), U32),
            vmem((7, S // 4, DC // 2), U32),
            vmem((H // 2 * WROWS + 32, D), U32),
            vmem((H * D, M), BF16),
            vmem((7, M // 2, M // 2), BF16),
            vmem((NTILE, S // 2, LANES), U32),
            vmem((2 * NTILE, HALO + S, LANES), F32),
            pltpu.SemaphoreType.DMA((11 + 3 * NKV + S // RA,)),
            pltpu.SemaphoreType.DMA((4,)),
        ],
        compiler_params=pltpu.CompilerParams(vmem_limit_bytes=126 * 2**20),
        name="fused_attn",
    )(
        A_x.reshape(S, M), A_c_kv.reshape(S, DC), A_w_q.reshape(M * H, D),
        A_w_uk.reshape(DC * H, D), A_w_uv.reshape(DC * H, D),
        A_w_o.reshape(H * D, M), B_x.reshape(S, M), B_wqkv, B_wo,
    )
    return out.reshape(1, S, 2 * M)
```

```python
import math

import jax
import jax.numpy as jnp
import numpy as np
from jax import lax
import jax.experimental.pallas as pl
import jax.experimental.pallas.tpu as pltpu

S = 2048
M = 1024
DC = 512
H = 32
D = 128
DH_B = 32
WIN, DIL = 8, 2
HALO = 16

LANES = 128
NTILE = M // LANES
BQ = 512
PM = 256
BM3 = 256
WROWS = M + 2 * DC
WPITCH = WROWS + 1
NKV = 8
NQB = 2
R1 = 128
PMA = 128
RA = 256
KS3 = 4
AFTER = True
ORDER = '01236789abcdef45'
AHEAD = 1
EARLY = True
CHAIN = True
R2 = 256
FRAC3 = 0.9

LOG2E = math.log2(math.e)
NT = (((1,), (1,)), ((), ()))
BF16 = jnp.bfloat16
F32 = jnp.float32
U32 = jnp.uint32


def _dot(a, b):
    return jnp.dot(a, b, preferred_element_type=F32)


def _dot_nt(a, b):
    return lax.dot_general(a, b, NT, preferred_element_type=F32)


def _recip(x):
    r = pltpu.reciprocal(x, approx=True)
    return r * (2.0 - x * r)


def _ds(start, size, align):
    if not isinstance(start, int):
        start = pl.multiple_of(start, align)
    return pl.ds(start, size)


class _SideWork:
    def __init__(self, step, ndots, *lists):
        keyed = [((i + 0.5) / len(l), j, f)
                 for j, l in enumerate(lists) for i, f in enumerate(l)]
        self.todo = sorted(keyed, key=lambda e: e[:2])
        self.ndots, self.dots, self.last, self.done = ndots, 0, None, None
        self.never = jnp.full((8, LANES), step) < 0

    def dot(self, a, b):
        y = _dot(a, b)
        self.dots += 1
        self.last = y[0:8, 0:LANES]
        while self.todo and self.todo[0][0] * self.ndots <= self.dots:
            self.done = self.todo.pop(0)[2]()
        return y

    def after(self, x):
        if self.done is None:
            return x
        done, self.done = pltpu.bitcast(self.done[0:8, 0:LANES], x.dtype), None
        return jnp.concatenate([jnp.where(self.never, done, x[:8]), x[8:]], axis=0)

    def pin(self, x):
        last = pltpu.bitcast(self.last, x.dtype)
        return jnp.concatenate([jnp.concatenate(
            [jnp.where(self.never, last, x[r:r + 8, c:c + LANES])
             for c in range(0, x.shape[1], LANES)], axis=1)
            for r in range(0, x.shape[0], 8)], axis=0)


def _low(u):
    return pltpu.bitcast(u << 16, F32)


def _high(u):
    return pltpu.bitcast(u & np.uint32(0xFFFF0000), F32)


def _words(x):
    return pltpu.bitcast(x, U32)


def _bf16(u):
    return pltpu.bitcast(u, BF16)


def _lhs_terms(a11, a12, a21, a22):
    return [a11 + a22, a21 + a22, a11, a22, a11 + a12, a21 - a11, a12 - a22]


def _rhs_terms(b11, b12, b21, b22):
    return [b11 + b22, b11, b12 - b22, b21 - b11, b22, b11 + b12, b21 + b22]


def _word_terms(terms, *blocks):
    lo, hi = [_low(u) for u in blocks], [_high(u) for u in blocks]
    out = []
    for a, b in zip(terms(*lo), terms(*hi)):
        plain = [u for u, l in zip(blocks, lo) if l is a]
        out.append(plain[0] if plain else _words(
            pltpu.pack_elementwise([a, b], packed_dtype=BF16)))
    return out


def _weave(a, b):
    return jnp.concatenate(
        [p[r:r + 16] for r in range(0, a.shape[0], 16) for p in (a, b)], axis=0)


def _combine(product, plain_first=False):
    if plain_first:
        c12, c21 = product(2), product(3)
        m = product(4)
        c11, c22, c12 = c21 - m, c12, c12 + m
        c11 = c11 + product(6)
        m = product(0)
        c11, c22 = c11 + m, c22 + m
        m = product(1)
        c21, c22 = c21 + m, c22 - m
        return _weave(c11, c21), _weave(c12, c22 + product(5))
    c22 = product(5)
    c12 = product(2)
    c22 = c22 + c12
    m = product(4)
    c12 = c12 + m
    c11 = product(6) - m
    m = product(0)
    c11, c22 = c11 + m, c22 + m
    c21 = product(3)
    c11 = c11 + c21
    m = product(1)
    c21, c22 = c21 + m, c22 - m
    return _weave(c11, c21), _weave(c12, c22)


def _kernel(xa_hbm, c_hbm, wq_hbm, wk_hbm, wv_hbm, woa_hbm, xb_hbm, wqkv_hbm,
            wob_hbm, out_hbm,
            xa_t, c_t, w_pair, woa, wob_t, qb_p, kvb, in_sem, out_sem):
    woa_copy = pltpu.make_async_copy(woa_hbm, woa, in_sem.at[10 + 3 * NKV])

    def phase1(xa, c, w_raw, xb, xb_t, wqkv, wkv_t, wob, wob_tmp, qb, tr_tmp):
        rr, xr = WROWS // NKV, S // NKV

        def xb_copy(i):
            rows = _ds(i * RA, RA, RA)
            return pltpu.make_async_copy(xb_hbm.at[rows], xb.at[rows],
                                         in_sem.at[11 + 3 * NKV + i])

        wq_b = [pltpu.make_async_copy(
            wqkv_hbm.at[:, c0:c0 + 512], wqkv.at[:, c0:c0 + 512],
            in_sem.at[4 + c0 // 512]) for c0 in (0, 512)]

        def wb_copies(i):
            rows = _ds(i * 512, 512, 512)
            return [
                pltpu.make_async_copy(wqkv_hbm.at[rows, M:3 * M],
                                      wqkv.at[rows, M:3 * M], in_sem.at[6 + i]),
                pltpu.make_async_copy(wob_hbm.at[rows], wob.at[rows],
                                      in_sem.at[8 + i])]

        def a_copies(i, w_src):
            rows = _ds(i * xr, xr, xr)
            return [
                pltpu.make_async_copy(w_src, w_raw.at[i], in_sem.at[10 + 3 * i]),
                pltpu.make_async_copy(xa_hbm.at[rows], xa.at[rows],
                                      in_sem.at[11 + 3 * i]),
                pltpu.make_async_copy(c_hbm.at[rows], c.at[rows],
                                      in_sem.at[12 + 3 * i])]

        w_srcs = [w.at[r * H:(r + rr) * H]
                  for w, n in ((wq_hbm, M), (wk_hbm, DC), (wv_hbm, DC))
                  for r in range(0, n, rr)]
        copies = ([wq_b[0]] + [xb_copy(i) for i in range(S // RA)] + [wq_b[1]] +
                  wb_copies(0) + wb_copies(1))
        for i, src in enumerate(w_srcs):
            copies += a_copies(i, src)
        for cp in copies + [woa_copy]:
            cp.start()

        def row_terms(src, dst, row0, pin):
            out = []
            for t in range(0, src.shape[1], 2 * LANES):
                top = _words(src[_ds(row0, 16, 16), t:t + 2 * LANES])
                bot = _words(src[_ds(row0 + 16, 16, 16), t:t + 2 * LANES])
                terms = _word_terms(_lhs_terms, pin(top[:, :LANES]), top[:, LANES:],
                                    bot[:, :LANES], pin(bot[:, LANES:]))
                for i, u in enumerate(terms):
                    dst[i, _ds(row0 // 4, 8, 8), t // 2:t // 2 + LANES] = u
                out.append(terms)
            return [jnp.concatenate(t, axis=1) for t in zip(*out)]

        def to_d_major(load, store, pin):
            def scatter(t):
                u = _words(load(t))
                ut = jnp.concatenate([pin(u[:8]), u[8:]], axis=0).T
                for j in range(LANES // DH_B):
                    tr_tmp[pl.ds(4 * t + j, DH_B, stride=H + 1), :] = (
                        ut[j * DH_B:(j + 1) * DH_B])

            def gather(t):
                v = jnp.concatenate(
                    [tr_tmp[pl.ds((4 * t + j) * (H + 1), H), :] for j in range(4)],
                    axis=0)
                store(t, v.T)
            return ([lambda t=t: scatter(t) for t in range(NTILE)] +
                    [lambda t=t: gather(t) for t in range(NTILE)])

        def weight_terms(left, right):
            def blocks(u, odd):
                return jnp.concatenate(
                    [u[r:r + 64] for r in range(64 * odd, u.shape[0], 128)], axis=0)
            return _word_terms(_rhs_terms, blocks(left, 0), blocks(right, 0),
                               blocks(left, 1), blocks(right, 1))

        def permute_w(part, r, pin):
            held = []

            def store(t, v):
                held.append(v)
                if t % 2:
                    for i, u in enumerate(weight_terms(*held[-2:])):
                        wkv_t[(part * NTILE + t) // 2, i, _ds(r // 4, 64, 64), :] = u
            c0 = (1 + part) * M
            return to_d_major(
                lambda t: wqkv[_ds(r, 256, 256), c0 + t * LANES:c0 + (t + 1) * LANES],
                store, pin)

        def permute_q(r, pin):
            def store(t, v):
                qb_p[t, _ds(r // 2, LANES, LANES), :] = v
            return to_d_major(lambda t: qb[t, _ds(r, 256, 256), :], store, pin)

        def project_pair(side, weight, store):
            for r in range(0, S // 2, R1):
                ys = _combine(lambda i: side.dot(
                    _bf16(xb_t[i, r // 2:(r + R1) // 2, :]), _bf16(weight(i))))
                for j, y in enumerate(ys):
                    store(j, 2 * r, y)

        ndots = 7 * S // (2 * R1)
        for t in range(2 * NTILE):
            kvb[t, 0:HALO, :] = jnp.zeros((HALO, LANES), F32)
        wq_b[0].wait()
        for p in range(2):
            w = _words(wqkv[:, p * 256:(p + 1) * 256])
            for i, u in enumerate(weight_terms(w[:, :LANES], w[:, LANES:])):
                wkv_t[NTILE + p, i] = u

        def q_step_a(i, carry):
            xb_copy(i).wait()
            for r in range(0, RA, 2 * R1):
                row0 = i * RA + r
                terms = [row_terms(xb, xb_t, row0 + g, lambda u: u)
                         for g in range(0, 2 * R1, 32)]
                terms = [jnp.concatenate(t, axis=0) for t in zip(*terms)]
                for p in range(2):
                    ys = _combine(lambda t: _dot(
                        _bf16(terms[t]), _bf16(wkv_t[NTILE + p, t])), p == 0 and r == 0)
                    for j, y in enumerate(ys):
                        qb[2 * p + j, _ds(row0, 2 * R1, 2 * R1), :] = y.astype(BF16)
            return carry

        lax.fori_loop(0, S // RA, q_step_a, 0)
        wq_b[1].wait()

        def q_step_b(i, carry):
            for cp in wb_copies(i):
                cp.wait()

            def scatter_wob(h):
                y = side.pin(wob[_ds(h * DH_B, DH_B, DH_B), :].astype(F32))
                for t in range(NTILE):
                    wob_tmp[t, pl.ds(h, DH_B, stride=H + 1), :] = (
                        y[:, t * LANES:(t + 1) * LANES])

            def store(j, r, y):
                qb[4 + 2 * i + j, r:r + 2 * R1, :] = y.astype(BF16)

            perm = []
            for part in range(2):
                for r in (0, 256):
                    perm += permute_w(part, i * 512 + r, lambda x: side.pin(x))
            side = _SideWork(
                i, ndots - 4, perm,
                [lambda j=j: scatter_wob(i * 16 + j) for j in range(16)])
            w = _words(wqkv[:, _ds(512 + i * 256, 256, 256)])
            w = weight_terms(w[:, :LANES], w[:, LANES:])
            project_pair(side, lambda t: w[t], store)
            return carry

        lax.fori_loop(0, NQB, q_step_b, 0)

        def kv_step(i, carry):
            for cp in a_copies(i, w_srcs[0]):
                cp.wait()

            def store(j, r, y):
                kvb[2 * i + j, HALO + r:HALO + r + 2 * R1, :] = y

            def split_pairs(r):
                v = side.pin(_words(w_raw[i, r * H:(r + 8) * H, :]))
                for m in range(8):
                    w_pair[pl.ds(i * rr + r + m, H // 2, stride=WPITCH), :] = (
                        v[m * H // 2:(m + 1) * H // 2])

            def wob_terms(d, c0):
                b = [side.pin(wob_tmp[t, pl.ds(e * (H + 1), H), :])
                     for e in (d, d + (DH_B // 2)) for t in (2 * c0, 2 * c0 + 1)]
                for j, y in enumerate(_rhs_terms(*b)):
                    wob_t[j, _ds(d * H, H, H), c0 * LANES:(c0 + 1) * LANES] = y.astype(BF16)

            nd = DH_B // 2 // NKV
            side = _SideWork(
                i, ndots - 4,
                [lambda r=r: split_pairs(r) for r in range(0, rr, 8)],
                permute_q(i * xr, lambda x: side.pin(x)),
                [lambda j=j, c0=c0: wob_terms(i * nd + j, c0)
                 for j in range(nd) for c0 in range(NTILE // 2)],
                [lambda r=r: row_terms(xa, xa_t, i * xr + r, side.pin)
                 for r in range(0, xr, 32)],
                [lambda r=r: row_terms(c, c_t, i * xr + r, side.pin)
                 for r in range(0, xr, 32)])
            project_pair(side, lambda t: wkv_t[i, t], store)
            return carry

        lax.fori_loop(0, NKV, kv_step, 0)

    pl.run_scoped(
        phase1,
        pltpu.VMEM((S, M), BF16),
        pltpu.VMEM((S, DC), BF16),
        pltpu.VMEM((NKV, WROWS // NKV * H, D), BF16),
        pltpu.VMEM((S, M), BF16),
        pltpu.VMEM((7, S // 4, M // 2), U32),
        pltpu.VMEM((M, 3 * M), BF16),
        pltpu.VMEM((NTILE + 2, 7, M // 4, LANES), U32),
        pltpu.VMEM((M, M), BF16),
        pltpu.VMEM((NTILE, DH_B * (H + 1), LANES), F32),
        pltpu.VMEM((NTILE, S, LANES), BF16),
        pltpu.VMEM((DH_B * (H + 1), LANES), U32),
    )
    woa_copy.wait()

    def phase23(ctx_t, woa_t, ks, vs, att_t, oa_buf, ob_buf):
        q_scale = D ** -0.5 * LOG2E

        def pair_step(pair, carry):
            def weight_terms(row0, n):
                top, bot = [jnp.concatenate(
                    [w_pair[pl.ds(pair * WPITCH + row0 + r, LANES), :]
                     for r in range(odd * LANES, n, 2 * LANES)], axis=0)
                    for odd in (0, 1)]
                return _rhs_terms(_low(top), _high(top), _low(bot), _high(bot))

            def out_weight_terms(r, t):
                top, bot = [_words(woa[_ds(pair * 2 * D + j * D + r, 16, 16),
                                       t * LANES:(t + 2) * LANES]) for j in range(2)]
                for i, u in enumerate(_word_terms(
                        _rhs_terms, side.pin(top[:, :LANES]), top[:, LANES:],
                        bot[:, :LANES], side.pin(bot[:, LANES:]))):
                    woa_t[t // 2, i, _ds((pair * D + r) // 2, 8, 8), :] = u

            side = _SideWork(
                pair, 7 * NTILE,
                [lambda r=r, t=t: out_weight_terms(r, t)
                 for r in range(0, D, 16) for t in range(0, NTILE, 2)])
            row = lax.broadcasted_iota(jnp.int32, (LANES, LANES), 0)
            col = lax.broadcasted_iota(jnp.int32, (LANES, LANES), 1)
            causal = col <= row
            never = jnp.full((LANES, LANES), pair) < 0
            wkv = [jnp.concatenate([a, b], axis=1).astype(BF16) for a, b in zip(
                weight_terms(M, DC), weight_terms(M + DC, DC))]
            wq = [a.astype(BF16) for a in weight_terms(0, M)]
            q, ctx = {}, {}

            def project_kv(g):
                kv = _combine(lambda i: side.dot(
                    _bf16(c_t[i, g * 64:(g + 1) * 64, :]), wkv[i]))
                for j in range(2):
                    ks[j, g * 256:(g + 1) * 256, :] = kv[j][:, :D].astype(BF16)
                    vs[j, g * 256:(g + 1) * 256, :] = kv[j][:, D:].astype(BF16)

            def project_q(g):
                ys = _combine(lambda i: _dot(
                    _bf16(xa_t[i, g * 64:(g + 1) * 64, :]), wq[i]))
                for j, y in enumerate(ys):
                    q[j, 2 * g] = y[:LANES] * q_scale
                    q[j, 2 * g + 1] = y[LANES:] * q_scale

            def scores(j, a):
                s = _dot_nt(q[j, a].astype(BF16), ks[j, 0:(a + 1) * LANES, :])
                s = [s[:, t * LANES:(t + 1) * LANES] for t in range(a + 1)]
                s[a] = jnp.where(causal, s[a], -1e30)
                return s

            def attend(j, a, s):
                m = s[0]
                for x in s[1:]:
                    m = jnp.maximum(m, x)
                m = jnp.max(m, axis=1, keepdims=True)
                p = [jnp.exp2(x - m) for x in s]
                total = p[0]
                for x in p[1:]:
                    total = total + x
                if a:
                    p[a] = jnp.where(never, total, p[a])
                o = _dot(jnp.concatenate(p, axis=1).astype(BF16),
                         vs[j, 0:(a + 1) * LANES, :])
                ctx[j, a] = o * _recip(jnp.sum(total, axis=1, keepdims=True))
                if j:
                    for r in range(0, LANES, 32):
                        terms = _lhs_terms(
                            ctx[0, a][r:r + 16], ctx[1, a][r:r + 16],
                            ctx[0, a][r + 16:r + 32], ctx[1, a][r + 16:r + 32])
                        dst = (a * LANES + r) // 2
                        for i, y in enumerate(terms):
                            ctx_t[i, pair, dst:dst + 16, :] = y.astype(BF16)

            strips = [(j, int(a, 16)) for a in ORDER for j in range(2)]
            kv_done, waiting = 0, None
            for n, (j, a) in enumerate(strips):
                while kv_done < min(NTILE, max(n + 1, a // 2 + 1)):
                    project_kv(kv_done)
                    kv_done += 1
                for key in strips[n:n + 1 + AHEAD]:
                    if key not in q:
                        project_q(key[1] // 2)
                s = scores(j, a)
                if waiting:
                    attend(*waiting)
                waiting = (j, a, s)
            attend(*waiting)
            return carry

        lax.fori_loop(0, H // 2, pair_step, 0)

        nblk = S // BM3
        b_scale = DH_B ** -0.5 * LOG2E

        def out_copies(i, slot):
            return [pltpu.make_async_copy(
                oa_buf.at[slot],
                out_hbm.at[_ds(i // 2 * 2 * BM3, 2 * BM3, BM3),
                           _ds(slot * (M // 2), M // 2, M // 2)],
                out_sem.at[5 * slot])] + [pltpu.make_async_copy(
                    ob_buf.at[n, slot],
                    out_hbm.at[_ds(i * BM3, BM3, BM3), M + n * 256:M + (n + 1) * 256],
                    out_sem.at[5 * slot + 1 + n]) for n in range(4)]

        def window_attention(r0, a, prev):
            n = 16
            pos = r0 + a + lax.broadcasted_iota(jnp.int32, (n, LANES), 0)
            q = [_bf16(qb_p[t, _ds((r0 + a) // 2, n // 2, 8), :]).astype(F32)
                 for t in range(NTILE)]
            if prev and CHAIN:
                q[0] = jnp.where(pos < 0, prev[-1][-1], q[0])
            src = [pl.ds(r0 + HALO + a - DIL * w, n) for w in range(WIN)]
            logits = []
            for w in range(WIN):
                l = q[0] * kvb[0, src[w], :]
                for t in range(1, NTILE):
                    l = l + q[t] * kvb[t, src[w], :]
                l = l + pltpu.roll(l, 2 * H, 1)
                l = (l + pltpu.roll(l, H, 1)) * b_scale
                if DIL * w > a:
                    l = jnp.where(pos >= DIL * w, l, -1e30)
                logits.append(l)
            m = logits[0]
            for l in logits[1:]:
                m = jnp.maximum(m, l)
            e = [jnp.exp2(l - m) for l in logits]
            total = e[0]
            for x in e[1:]:
                total = total + x
            inv = _recip(total)
            e = [x * inv for x in e]
            o = []
            for t in range(NTILE):
                acc = e[0] * kvb[NTILE + t, src[0], :]
                for w in range(1, WIN):
                    acc = acc + e[w] * kvb[NTILE + t, src[w], :]
                o.append(acc)
            prev.append(o)
            if a % 32:
                blocks = [jnp.concatenate(x, axis=1)
                          for o in prev[-2:] for x in (o[:NTILE // 2], o[NTILE // 2:])]
                for i, y in enumerate(_lhs_terms(*blocks)):
                    att_t[i, a // 32 * 16:a // 32 * 16 + 16, :] = y.astype(BF16)
            return o[-1] if AFTER else None

        def out_step(i, carry):
            slot = i % 2
            r0 = pl.multiple_of(i * BM3, BM3)

            @pl.when(i >= 2)
            def _():
                for cp in out_copies(i - 2, slot):
                    cp.wait()

            prev = []
            side = _SideWork(
                i, int(FRAC3 * 7 * 2 * KS3),
                [lambda a=a: window_attention(r0, a, prev) for a in range(0, BM3, 16)])
            rows = _ds(i // 2 * BM3, BM3, BM3)

            def product(n, t):
                y = None
                np_ = H // 2 // KS3
                for k in range(0, H // 2, np_):
                    part = side.dot(
                        jnp.concatenate(
                            [ctx_t[t, p, rows, :] for p in range(k, k + np_)], axis=1),
                        _bf16(side.after(woa_t[2 * slot + n, t, k * D // 2:(k + np_) * D // 2, :])))
                    y = part if y is None else y + part
                return y

            for n in range(2):
                for j, y in enumerate(_combine(lambda t: product(n, t))):
                    oa_buf[slot, :, (2 * n + j) * LANES:(2 * n + j + 1) * LANES] = (
                        y.astype(BF16))
            copies = out_copies(i, slot)
            if EARLY:
                copies[0].start()
            for n in range(4):
                ys = _combine(
                    lambda t: _dot(att_t[t], wob_t[t, :, n * LANES:(n + 1) * LANES]))
                ob_buf[n, slot] = jnp.concatenate(ys, axis=1).astype(BF16)
                if EARLY:
                    copies[1 + n].start()
            if not EARLY:
                for cp in copies:
                    cp.start()
            return carry

        lax.fori_loop(0, nblk, out_step, 0)
        for i in (nblk - 2, nblk - 1):
            for cp in out_copies(i, i % 2):
                cp.wait()

    pl.run_scoped(
        phase23,
        pltpu.VMEM((7, H // 2, S // 2, D), BF16),
        pltpu.VMEM((NTILE // 2, 7, H * D // 4, LANES), U32),
        pltpu.VMEM((2, S, D), BF16),
        pltpu.VMEM((2, S, D), BF16),
        pltpu.VMEM((7, BM3 // 2, M // 2), BF16),
        pltpu.VMEM((2, 2 * BM3, M // 2), BF16),
        pltpu.VMEM((4, 2, BM3, M // 4), BF16),
    )


@jax.jit
def pallas_concat_heads__compressed_kv_cla__sliding_local_dilated__prompt_kernel(
    A_x: jax.Array,
    A_c_kv: jax.Array,
    A_w_q: jax.Array,
    A_w_uk: jax.Array,
    A_w_uv: jax.Array,
    A_w_o: jax.Array,
    B_x: jax.Array,
    B_wqkv: jax.Array,
    B_wo: jax.Array,
):
    vmem = pltpu.VMEM
    out = pl.pallas_call(
        _kernel,
        out_shape=jax.ShapeDtypeStruct((S, 2 * M), BF16),
        in_specs=[pl.BlockSpec(memory_space=pl.ANY)] * 9,
        out_specs=pl.BlockSpec(memory_space=pl.ANY),
        scratch_shapes=[
            vmem((7, S // 4, M // 2), U32),
            vmem((7, S // 4, DC // 2), U32),
            vmem((H // 2 * WROWS + 32, D), U32),
            vmem((H * D, M), BF16),
            vmem((7, M // 2, M // 2), BF16),
            vmem((NTILE, S // 2, LANES), U32),
            vmem((2 * NTILE, HALO + S, LANES), F32),
            pltpu.SemaphoreType.DMA((11 + 3 * NKV + S // RA,)),
            pltpu.SemaphoreType.DMA((10,)),
        ],
        compiler_params=pltpu.CompilerParams(vmem_limit_bytes=126 * 2**20),
        name="fused_attn",
    )(
        A_x.reshape(S, M), A_c_kv.reshape(S, DC), A_w_q.reshape(M * H, D),
        A_w_uk.reshape(DC * H, D), A_w_uv.reshape(DC * H, D),
        A_w_o.reshape(H * D, M), B_x.reshape(S, M), B_wqkv, B_wo,
    )
    return out.reshape(1, S, 2 * M)
```

```python
import math

import jax
import jax.numpy as jnp
import numpy as np
from jax import lax
import jax.experimental.pallas as pl
import jax.experimental.pallas.tpu as pltpu

S = 2048
M = 1024
DC = 512
H = 32
D = 128
DH_B = 32
WIN, DIL = 8, 2
HALO = 16

LANES = 128
NTILE = M // LANES
BQ = 512
PM = 256
BM3 = 256
WROWS = M + 2 * DC
WPITCH = WROWS + 1
NKV = 8
NQB = 2
R1 = 128
PMA = 128
RA = 256
KS3 = 4
AFTER = True
ORDER = '01235489abcdfe67'
AHEAD = 3
KRATE = 1
SPL = 4
KVS = 4
QBS = 4
FIRST = (4, 1, 2, 3, 6, 0, 5)
PULLS = 1
KEEP = 48
PULL = 1
PULLAT = 1
KAH = 1
QSIDE = 1
WOD = 28
JOUT = 1
QMID = False
ONLY = ''
EARLY = True
CHAIN = False
R2 = 256
FRAC3 = 0.9

LOG2E = math.log2(math.e)
NT = (((1,), (1,)), ((), ()))
BF16 = jnp.bfloat16
F32 = jnp.float32
U32 = jnp.uint32


def _dot(a, b):
    return jnp.dot(a, b, preferred_element_type=F32)


def _dot_nt(a, b):
    return lax.dot_general(a, b, NT, preferred_element_type=F32)


def _recip(x):
    r = pltpu.reciprocal(x, approx=True)
    return r * (2.0 - x * r)


def _ds(start, size, align):
    if not isinstance(start, int):
        start = pl.multiple_of(start, align)
    return pl.ds(start, size)


class _SideWork:
    def __init__(self, step, ndots, *lists):
        keyed = [((i + 0.5) / len(l), j, f)
                 for j, l in enumerate(lists) for i, f in enumerate(l)]
        self.todo = sorted(keyed, key=lambda e: e[:2])
        self.ndots, self.dots, self.last, self.done = ndots, 0, None, None
        self.never = jnp.full((8, LANES), step) < 0

    def dot(self, a, b):
        y = _dot(a, b)
        self.dots += 1
        self.last = y[0:8, 0:LANES]
        while self.todo and self.todo[0][0] * self.ndots <= self.dots:
            self.done = self.todo.pop(0)[2]()
        return y

    def after(self, x):
        if self.done is None:
            return x
        done, self.done = pltpu.bitcast(self.done[0:8, 0:LANES], x.dtype), None
        return jnp.concatenate([jnp.where(self.never, done, x[:8]), x[8:]], axis=0)

    def pin(self, x):
        last = pltpu.bitcast(self.last, x.dtype)
        return jnp.concatenate([jnp.concatenate(
            [jnp.where(self.never, last, x[r:r + 8, c:c + LANES])
             for c in range(0, x.shape[1], LANES)], axis=1)
            for r in range(0, x.shape[0], 8)], axis=0)


def _low(u):
    return pltpu.bitcast(u << 16, F32)


def _high(u):
    return pltpu.bitcast(u & np.uint32(0xFFFF0000), F32)


def _words(x):
    return pltpu.bitcast(x, U32)


def _bf16(u):
    return pltpu.bitcast(u, BF16)


def _lhs_terms(a11, a12, a21, a22):
    return [a11 + a22, a21 + a22, a11, a22, a11 + a12, a21 - a11, a12 - a22]


def _rhs_terms(b11, b12, b21, b22):
    return [b11 + b22, b11, b12 - b22, b21 - b11, b22, b11 + b12, b21 + b22]


def _word_terms(terms, *blocks):
    lo, hi = [_low(u) for u in blocks], [_high(u) for u in blocks]
    out = []
    for a, b in zip(terms(*lo), terms(*hi)):
        plain = [u for u, l in zip(blocks, lo) if l is a]
        out.append(plain[0] if plain else _words(
            pltpu.pack_elementwise([a, b], packed_dtype=BF16)))
    return out


def _weave(a, b):
    return jnp.concatenate(
        [p[r:r + 16] for r in range(0, a.shape[0], 16) for p in (a, b)], axis=0)


def _combine(product, order=(5, 2, 4, 6, 0, 3, 1)):
    signs = ((1, 0, 0, 1), (0, 0, 1, -1), (0, 1, 0, 1), (1, 0, 1, 0),
             (-1, 1, 0, 0), (0, 0, 0, 1), (1, 0, 0, 0))
    plus, minus = [None] * 4, [None] * 4
    for i in order:
        m = product(i)
        for j, sign in enumerate(signs[i]):
            if sign > 0:
                plus[j] = m if plus[j] is None else plus[j] + m
            elif sign < 0:
                minus[j] = m
            if plus[j] is not None and minus[j] is not None:
                plus[j], minus[j] = plus[j] - minus[j], None
    c11, c12, c21, c22 = plus
    return _weave(c11, c21), _weave(c12, c22)


def _kernel(xa_hbm, c_hbm, wq_hbm, wk_hbm, wv_hbm, woa_hbm, xb_hbm, wqkv_hbm,
            wob_hbm, out_hbm,
            xa_t, c_t, w_pair, woa, wob_t, qb_p, kvb, in_sem, out_sem):
    woa_copy = pltpu.make_async_copy(woa_hbm, woa, in_sem.at[10 + 3 * NKV])

    def phase1(xa, c, w_raw, xb, xb_t, wqkv, wkv_t, wob, wob_tmp, qb, tr_tmp):
        rr, xr = WROWS // NKV, S // NKV

        def xb_copy(i):
            rows = _ds(i * RA, RA, RA)
            return pltpu.make_async_copy(xb_hbm.at[rows], xb.at[rows],
                                         in_sem.at[11 + 3 * NKV + i])

        wq_b = [pltpu.make_async_copy(
            wqkv_hbm.at[:, c0:c0 + 512], wqkv.at[:, c0:c0 + 512],
            in_sem.at[4 + c0 // 512]) for c0 in (0, 512)]

        def wb_copies(i):
            rows = _ds(i * 512, 512, 512)
            return [
                pltpu.make_async_copy(wqkv_hbm.at[rows, M:3 * M],
                                      wqkv.at[rows, M:3 * M], in_sem.at[6 + i]),
                pltpu.make_async_copy(wob_hbm.at[rows], wob.at[rows],
                                      in_sem.at[8 + i])]

        def a_copies(i, w_src):
            rows = _ds(i * xr, xr, xr)
            return [
                pltpu.make_async_copy(w_src, w_raw.at[i], in_sem.at[10 + 3 * i]),
                pltpu.make_async_copy(xa_hbm.at[rows], xa.at[rows],
                                      in_sem.at[11 + 3 * i]),
                pltpu.make_async_copy(c_hbm.at[rows], c.at[rows],
                                      in_sem.at[12 + 3 * i])]

        w_srcs = [w.at[r * H:(r + rr) * H]
                  for w, n in ((wq_hbm, M), (wk_hbm, DC), (wv_hbm, DC))
                  for r in range(0, n, rr)]
        copies = ([wq_b[0]] + [xb_copy(i) for i in range(S // RA)] + [wq_b[1]] +
                  wb_copies(0) + wb_copies(1))
        for i, src in enumerate(w_srcs):
            copies += a_copies(i, src)
        for cp in copies + [woa_copy]:
            cp.start()

        def row_terms(src, dst, row0, t, pin=lambda u: u):
            top = _words(src[_ds(row0, 16, 16), t:t + 2 * LANES])
            bot = _words(src[_ds(row0 + 16, 16, 16), t:t + 2 * LANES])
            terms = _word_terms(_lhs_terms, pin(top[:, :LANES]), top[:, LANES:],
                                bot[:, :LANES], pin(bot[:, LANES:]))
            for i, u in enumerate(terms):
                dst[i, _ds(row0 // 4, 8, 8), t // 2:t // 2 + LANES] = u
            return terms

        def to_d_major(load, store, pin):
            def scatter(t):
                u = _words(load(t))
                ut = jnp.concatenate([pin(u[:8]), u[8:]], axis=0).T
                for j in range(LANES // DH_B):
                    tr_tmp[pl.ds(4 * t + j, DH_B, stride=H + 1), :] = (
                        ut[j * DH_B:(j + 1) * DH_B])

            def gather(t):
                v = jnp.concatenate(
                    [tr_tmp[pl.ds((4 * t + j) * (H + 1), H), :] for j in range(4)],
                    axis=0)
                store(t, v.T)
            return ([lambda t=t: scatter(t) for t in range(NTILE)] +
                    [lambda t=t: gather(t) for t in range(NTILE)])

        def weight_terms(left, right):
            def blocks(u, odd):
                return jnp.concatenate(
                    [u[r:r + 64] for r in range(64 * odd, u.shape[0], 128)], axis=0)
            return _word_terms(_rhs_terms, blocks(left, 0), blocks(right, 0),
                               blocks(left, 1), blocks(right, 1))

        def permute_w(part, r, pin):
            held = []

            def store(t, v):
                held.append(v)
                if t % 2:
                    for i, u in enumerate(weight_terms(*held[-2:])):
                        wkv_t[(part * NTILE + t) // 2, i, _ds(r // 4, 64, 64), :] = u
            c0 = (1 + part) * M
            return to_d_major(
                lambda t: wqkv[_ds(r, 256, 256), c0 + t * LANES:c0 + (t + 1) * LANES],
                store, pin)

        def permute_q(r, pin):
            def store(t, v):
                qb_p[t, _ds(r // 2, LANES, LANES), :] = v
            return to_d_major(lambda t: qb[t, _ds(r, 256, 256), :], store, pin)

        def project_pair(side, weight, store):
            for r in range(0, S // 2, R1):
                ys = _combine(lambda i: side.dot(
                    _bf16(xb_t[i, r // 2:(r + R1) // 2, :]), _bf16(weight(i))))
                for j, y in enumerate(ys):
                    store(j, 2 * r, y)

        ndots = 7 * S // (2 * R1)
        for t in range(2 * NTILE):
            kvb[t, 0:HALO, :] = jnp.zeros((HALO, LANES), F32)
        wq_b[0].wait()
        for p in range(2):
            w = _words(wqkv[:, p * 256:(p + 1) * 256])
            for i, u in enumerate(weight_terms(w[:, :LANES], w[:, LANES:])):
                wkv_t[NTILE + p, i] = u

        def q_step_a(i, carry):
            xb_copy(i).wait()
            for r in range(0, RA, 2 * R1):
                row0 = i * RA + r
                terms = [[row_terms(xb, xb_t, row0 + g, t) for t in range(0, M, 256)]
                         for g in range(0, 2 * R1, 32)]
                terms = [jnp.concatenate(
                    [jnp.concatenate([u[k] for u in row], axis=1) for row in terms],
                    axis=0) for k in range(7)]
                for p in range(2):
                    ys = _combine(lambda t: _dot(
                        _bf16(terms[t]), _bf16(wkv_t[NTILE + p, t])), *([(2, 3, 4, 6, 0, 1, 5)] if p == 0 and r == 0 else []))
                    for j, y in enumerate(ys):
                        qb[2 * p + j, _ds(row0, 2 * R1, 2 * R1), :] = y.astype(BF16)
            return carry

        if ONLY in ('', 'qa'): lax.fori_loop(0, S // RA, q_step_a, 0)
        wq_b[1].wait()

        def q_step_b(i, carry):
            for cp in wb_copies(i):
                cp.wait()

            def scatter_wob(h):
                y = side.pin(wob[_ds(h * DH_B, DH_B, DH_B), :].astype(F32))
                for t in range(NTILE):
                    wob_tmp[t, pl.ds(h, DH_B, stride=H + 1), :] = (
                        y[:, t * LANES:(t + 1) * LANES])

            def store(j, r, y):
                qb[4 + 2 * i + j, r:r + 2 * R1, :] = y.astype(BF16)

            perm = []
            for part in range(2):
                for r in (0, 256):
                    perm += permute_w(part, i * 512 + r, lambda x: side.pin(x))
            side = _SideWork(
                i, ndots - QBS, perm,
                [lambda j=j: scatter_wob(i * 16 + j) for j in range(16)])
            w = _words(wqkv[:, _ds(512 + i * 256, 256, 256)])
            w = weight_terms(w[:, :LANES], w[:, LANES:])
            project_pair(side, lambda t: w[t], store)
            return carry

        if ONLY in ('', 'qb'): lax.fori_loop(0, NQB, q_step_b, 0)

        def kv_step(i, carry):
            for cp in a_copies(i, w_srcs[0]):
                cp.wait()

            def store(j, r, y):
                kvb[2 * i + j, HALO + r:HALO + r + 2 * R1, :] = y

            def split_pairs(r):
                v = side.pin(_words(w_raw[i, r * H:(r + SPL) * H, :]))
                for m in range(SPL):
                    w_pair[pl.ds(i * rr + r + m, H // 2, stride=WPITCH), :] = (
                        v[m * H // 2:(m + 1) * H // 2])

            def wob_terms(d, c0):
                b = [side.pin(wob_tmp[t, pl.ds(e * (H + 1), H), :])
                     for e in (d, d + (DH_B // 2)) for t in (2 * c0, 2 * c0 + 1)]
                for j, y in enumerate(_rhs_terms(*b)):
                    wob_t[j, _ds(d * H, H, H), c0 * LANES:(c0 + 1) * LANES] = y.astype(BF16)

            nd = DH_B // 2 // NKV
            side = _SideWork(
                i, ndots - KVS,
                [lambda r=r: split_pairs(r) for r in range(0, rr, SPL)],
                permute_q(i * xr, lambda x: side.pin(x)),
                [lambda j=j, c0=c0: wob_terms(i * nd + j, c0)
                 for j in range(nd) for c0 in range(NTILE // 2)],
                [lambda r=r, t=t, a=a: row_terms(*a, i * xr + r, t, side.pin)[0]
                 for r in range(0, xr, 32) for a in ((xa, xa_t), (c, c_t))
                 for t in range(0, a[0].shape[1], 256)])
            project_pair(side, lambda t: wkv_t[i, t], store)
            return carry

        if ONLY in ('', 'qb', 'kv'): lax.fori_loop(0, NKV, kv_step, 0)

    pl.run_scoped(
        phase1,
        pltpu.VMEM((S, M), BF16),
        pltpu.VMEM((S, DC), BF16),
        pltpu.VMEM((NKV, WROWS // NKV * H, D), BF16),
        pltpu.VMEM((S, M), BF16),
        pltpu.VMEM((7, S // 4, M // 2), U32),
        pltpu.VMEM((M, 3 * M), BF16),
        pltpu.VMEM((NTILE + 2, 7, M // 4, LANES), U32),
        pltpu.VMEM((M, M), BF16),
        pltpu.VMEM((NTILE, DH_B * (H + 1), LANES), F32),
        pltpu.VMEM((NTILE, S, LANES), BF16),
        pltpu.VMEM((DH_B * (H + 1), LANES), U32),
    )
    woa_copy.wait()

    def phase23(ctx_t, woa_t, ks, vs, att_t, oa_buf, ob_buf):
        q_scale = D ** -0.5 * LOG2E

        def pair_step(pair, carry):
            def weight_terms(row0, n):
                top, bot = [jnp.concatenate(
                    [w_pair[pl.ds(pair * WPITCH + row0 + r, LANES), :]
                     for r in range(odd * LANES, n, 2 * LANES)], axis=0)
                    for odd in (0, 1)]
                return _rhs_terms(_low(top), _high(top), _low(bot), _high(bot))

            def out_weight_terms(r, t):
                top, bot = [_words(woa[_ds(pair * 2 * D + j * D + r, 16, 16),
                                       t * LANES:(t + 2) * LANES]) for j in range(2)]
                for i, u in enumerate(_word_terms(
                        _rhs_terms, side.pin(top[:, :LANES]), top[:, LANES:],
                        bot[:, :LANES], side.pin(bot[:, LANES:]))):
                    woa_t[t // 2, i, _ds((pair * D + r) // 2, 8, 8), :] = u

            side = _SideWork(
                pair, WOD,
                [lambda r=r, t=t: out_weight_terms(r, t)
                 for r in range(0, D, 16) for t in range(0, NTILE, 2)])
            row = lax.broadcasted_iota(jnp.int32, (LANES, LANES), 0)
            col = lax.broadcasted_iota(jnp.int32, (LANES, LANES), 1)
            causal = col <= row
            never = jnp.full((LANES, LANES), pair) < 0
            wkv = [jnp.concatenate([a, b], axis=1).astype(BF16) for a, b in zip(
                weight_terms(M, DC), weight_terms(M + DC, DC))]
            wq = [a.astype(BF16) for a in weight_terms(0, M)]
            q, ctx, finished = {}, {}, []

            def project_kv(g):
                kv = _combine(lambda i: (_dot if QSIDE else side.dot)(
                    _bf16(c_t[i, g * 64:(g + 1) * 64, :]), wkv[i]),
                    *([FIRST] if g == 0 else []))
                for j in range(2):
                    ks[j, g * 256:(g + 1) * 256, :] = kv[j][:, :D].astype(BF16)
                    vs[j, g * 256:(g + 1) * 256, :] = kv[j][:, D:].astype(BF16)

            def project_q(g):
                def product(i):
                    x = xa_t[i, g * 64:(g + 1) * 64, :]
                    if PULL and not PULLS and i == PULLAT and len(finished) > KEEP:
                        y = finished.pop(0)
                        while len(finished) > KEEP:
                            y = jnp.maximum(y, finished.pop(0))
                        x = jnp.concatenate([jnp.concatenate(
                            [jnp.where(never[:8], _words(y), x[:8, :LANES]), x[:8, LANES:]],
                            axis=1), x[8:]], axis=0)
                    return (side.dot if QSIDE else _dot)(_bf16(x), wq[i])
                ys = _combine(product)
                for j, y in enumerate(ys):
                    q[j, 2 * g] = y[:LANES] * q_scale
                    q[j, 2 * g + 1] = y[LANES:] * q_scale

            def scores(j, a):
                x = q[j, a]
                if PULLS and len(finished) > KEEP:
                    y = finished.pop(0)
                    while len(finished) > KEEP:
                        y = jnp.maximum(y, finished.pop(0))
                    x = jnp.concatenate([x[:-8], jnp.where(never[:8], y, x[-8:])], axis=0)
                s = _dot_nt(x.astype(BF16), ks[j, 0:(a + 1) * LANES, :])
                s = [s[:, t * LANES:(t + 1) * LANES] for t in range(a + 1)]
                s[a] = jnp.where(causal, s[a], -1e30)
                return s

            def attend(j, a, s):
                m = s[0]
                for x in s[1:]:
                    m = jnp.maximum(m, x)
                m = jnp.max(m, axis=1, keepdims=True)
                p = [jnp.exp2(x - m) for x in s]
                total = p[0]
                for x in p[1:]:
                    total = total + x
                if a:
                    p[a] = jnp.where(never, total, p[a])
                o = _dot(jnp.concatenate(p, axis=1).astype(BF16),
                         vs[j, 0:(a + 1) * LANES, :])
                inv = _recip(jnp.sum(total, axis=1, keepdims=True))
                if PULL & 4:
                    finished.extend(jnp.broadcast_to(inv[r:r + 8], (8, LANES)) for r in range(0, LANES, 8))
                ctx[j, a] = o * inv
                if PULL & 1:
                    finished.extend(ctx[j, a][r:r + 8] for r in range(0, LANES, 8))
                if j:
                    for r in range(0, LANES, 32):
                        terms = _lhs_terms(
                            ctx[0, a][r:r + 16], ctx[1, a][r:r + 16],
                            ctx[0, a][r + 16:r + 32], ctx[1, a][r + 16:r + 32])
                        dst = (a * LANES + r) // 2
                        for i, y in enumerate(terms):
                            ctx_t[i, pair, dst:dst + 16, :] = y.astype(BF16)
                            if PULL & 2:
                                finished.append(ctx_t[i, pair, dst:dst + 16, :].astype(F32)[:8])

            strips = [(j, int(a, 16)) for a in ORDER for j in range(2)]
            if JOUT:
                strips = [(j, int(ORDER[g + e], 16)) for g in range(0, 16, 2) for j in range(2) for e in range(2)]
            kv_done, waiting = 0, None
            for n, (j, a) in enumerate(strips):
                while kv_done < min(NTILE, max(1 + int(n * KRATE), max(x[1] for x in strips[:n + 1 + KAH]) // 2 + 1)):
                    project_kv(kv_done)
                    kv_done += 1
                if (j, a) not in q:
                    project_q(a // 2)
                if QMID:
                    s = scores(j, a)
                for key in strips[n:n + 1 + AHEAD]:
                    if key not in q:
                        project_q(key[1] // 2)
                if not QMID:
                    s = scores(j, a)
                if waiting:
                    attend(*waiting)
                waiting = (j, a, s)
            attend(*waiting)
            return carry

        if ONLY in ('', 'pair', 'kv'): lax.fori_loop(0, H // 2, pair_step, 0)

        nblk = S // BM3
        b_scale = DH_B ** -0.5 * LOG2E

        def out_copies(i, slot):
            return [pltpu.make_async_copy(
                oa_buf.at[slot],
                out_hbm.at[_ds(i // 2 * 2 * BM3, 2 * BM3, BM3),
                           _ds(slot * (M // 2), M // 2, M // 2)],
                out_sem.at[5 * slot])] + [pltpu.make_async_copy(
                    ob_buf.at[n, slot],
                    out_hbm.at[_ds(i * BM3, BM3, BM3), M + n * 256:M + (n + 1) * 256],
                    out_sem.at[5 * slot + 1 + n]) for n in range(4)]

        def window_attention(r0, a, prev):
            n = 16
            pos = r0 + a + lax.broadcasted_iota(jnp.int32, (n, LANES), 0)
            q = [_bf16(qb_p[t, _ds((r0 + a) // 2, n // 2, 8), :]).astype(F32)
                 for t in range(NTILE)]
            if prev and CHAIN:
                q[0] = jnp.where(pos < 0, prev[-1][-1], q[0])
            src = [pl.ds(r0 + HALO + a - DIL * w, n) for w in range(WIN)]
            logits = []
            for w in range(WIN):
                l = q[0] * kvb[0, src[w], :]
                for t in range(1, NTILE):
                    l = l + q[t] * kvb[t, src[w], :]
                l = l + pltpu.roll(l, 2 * H, 1)
                l = (l + pltpu.roll(l, H, 1)) * b_scale
                if DIL * w > a:
                    l = jnp.where(pos >= DIL * w, l, -1e30)
                logits.append(l)
            m = logits[0]
            for l in logits[1:]:
                m = jnp.maximum(m, l)
            e = [jnp.exp2(l - m) for l in logits]
            total = e[0]
            for x in e[1:]:
                total = total + x
            inv = _recip(total)
            e = [x * inv for x in e]
            o = []
            for t in range(NTILE):
                acc = e[0] * kvb[NTILE + t, src[0], :]
                for w in range(1, WIN):
                    acc = acc + e[w] * kvb[NTILE + t, src[w], :]
                o.append(acc)
            prev.append(o)
            if a % 32:
                blocks = [jnp.concatenate(x, axis=1)
                          for o in prev[-2:] for x in (o[:NTILE // 2], o[NTILE // 2:])]
                for i, y in enumerate(_lhs_terms(*blocks)):
                    att_t[i, a // 32 * 16:a // 32 * 16 + 16, :] = y.astype(BF16)
            return o[-1] if AFTER else None

        def out_step(i, carry):
            slot = i % 2
            r0 = pl.multiple_of(i * BM3, BM3)

            @pl.when(i >= 2)
            def _():
                for cp in out_copies(i - 2, slot):
                    cp.wait()

            prev = []
            side = _SideWork(
                i, int(FRAC3 * 7 * 2 * KS3),
                [lambda a=a: window_attention(r0, a, prev) for a in range(0, BM3, 16)])
            rows = _ds(i // 2 * BM3, BM3, BM3)

            def product(n, t):
                y = None
                np_ = H // 2 // KS3
                for k in range(0, H // 2, np_):
                    part = side.dot(
                        jnp.concatenate(
                            [ctx_t[t, p, rows, :] for p in range(k, k + np_)], axis=1),
                        _bf16(side.after(woa_t[2 * slot + n, t, k * D // 2:(k + np_) * D // 2, :])))
                    y = part if y is None else y + part
                return y

            for n in range(2):
                for j, y in enumerate(_combine(lambda t: product(n, t))):
                    oa_buf[slot, :, (2 * n + j) * LANES:(2 * n + j + 1) * LANES] = (
                        y.astype(BF16))
            copies = out_copies(i, slot)
            if EARLY:
                copies[0].start()
            for n in range(4):
                ys = _combine(
                    lambda t: _dot(att_t[t], wob_t[t, :, n * LANES:(n + 1) * LANES]))
                ob_buf[n, slot] = jnp.concatenate(ys, axis=1).astype(BF16)
                if EARLY:
                    copies[1 + n].start()
            if not EARLY:
                for cp in copies:
                    cp.start()
            return carry

        if ONLY in ('', 'out', 'kv'): lax.fori_loop(0, nblk, out_step, 0)
        else:
            def fin(h, c):
                oa_buf[0, 0:16, 0:128] = ctx_t[h, h, _ds(h*16, 16, 16), :] + _bf16(woa_t[h, h, _ds(h*8, 8, 8), :])
                return c
            lax.fori_loop(0, 4, fin, 0)
        for i in (nblk - 2, nblk - 1):
            for cp in out_copies(i, i % 2):
                cp.wait()

    pl.run_scoped(
        phase23,
        pltpu.VMEM((7, H // 2, S // 2, D), BF16),
        pltpu.VMEM((NTILE // 2, 7, H * D // 4, LANES), U32),
        pltpu.VMEM((2, S, D), BF16),
        pltpu.VMEM((2, S, D), BF16),
        pltpu.VMEM((7, BM3 // 2, M // 2), BF16),
        pltpu.VMEM((2, 2 * BM3, M // 2), BF16),
        pltpu.VMEM((4, 2, BM3, M // 4), BF16),
    )


@jax.jit
def pallas_concat_heads__compressed_kv_cla__sliding_local_dilated__prompt_kernel(
    A_x: jax.Array,
    A_c_kv: jax.Array,
    A_w_q: jax.Array,
    A_w_uk: jax.Array,
    A_w_uv: jax.Array,
    A_w_o: jax.Array,
    B_x: jax.Array,
    B_wqkv: jax.Array,
    B_wo: jax.Array,
):
    vmem = pltpu.VMEM
    out = pl.pallas_call(
        _kernel,
        out_shape=jax.ShapeDtypeStruct((S, 2 * M), BF16),
        in_specs=[pl.BlockSpec(memory_space=pl.ANY)] * 9,
        out_specs=pl.BlockSpec(memory_space=pl.ANY),
        scratch_shapes=[
            vmem((7, S // 4, M // 2), U32),
            vmem((7, S // 4, DC // 2), U32),
            vmem((H // 2 * WROWS + 32, D), U32),
            vmem((H * D, M), BF16),
            vmem((7, M // 2, M // 2), BF16),
            vmem((NTILE, S // 2, LANES), U32),
            vmem((2 * NTILE, HALO + S, LANES), F32),
            pltpu.SemaphoreType.DMA((11 + 3 * NKV + S // RA,)),
            pltpu.SemaphoreType.DMA((10,)),
        ],
        compiler_params=pltpu.CompilerParams(vmem_limit_bytes=126 * 2**20),
        name="fused_attn",
    )(
        A_x.reshape(S, M), A_c_kv.reshape(S, DC), A_w_q.reshape(M * H, D),
        A_w_uk.reshape(DC * H, D), A_w_uv.reshape(DC * H, D),
        A_w_o.reshape(H * D, M), B_x.reshape(S, M), B_wqkv, B_wo,
    )
    return out.reshape(1, S, 2 * M)
```

```python
import math

import jax
import jax.numpy as jnp
import numpy as np
from jax import lax
import jax.experimental.pallas as pl
import jax.experimental.pallas.tpu as pltpu

S = 2048
M = 1024
DC = 512
H = 32
D = 128
DB = 32
WIN, DIL = 8, 2
HALO = 16

LANES = 128
NTILE = M // LANES
BM = 256
NBM = S // BM
WROWS = M + 2 * DC
WPITCH = WROWS + 1
BPITCH = H + 1
STRIPS = ((0, 1), (2, 3), (5, 4), (8, 9), (10, 11), (12, 13), (15, 14), (6, 7))

LOG2E = math.log2(math.e)
BF16 = jnp.bfloat16
F32 = jnp.float32
U32 = jnp.uint32


def _dot(a, b):
    return jnp.dot(a, b, preferred_element_type=F32)


def _dot_nt(a, b):
    return lax.dot_general(a, b, (((1,), (1,)), ((), ())),
                           preferred_element_type=F32)


def _recip(x):
    r = pltpu.reciprocal(x, approx=True)
    return r * (2.0 - x * r)


def _fold(op, xs):
    y = xs[0]
    for x in xs[1:]:
        y = op(y, x)
    return y


def _ds(start, size, align):
    if not isinstance(start, int):
        start = pl.multiple_of(start, align)
    return pl.ds(start, size)


def _words(x):
    return pltpu.bitcast(x, U32)


def _bf16(u):
    return pltpu.bitcast(u, BF16)


def _low(u):
    return pltpu.bitcast(u << 16, F32)


def _high(u):
    return pltpu.bitcast(u & np.uint32(0xFFFF0000), F32)


def _lhs_terms(a11, a12, a21, a22):
    return [a11 + a22, a21 + a22, a11, a22, a11 + a12, a21 - a11, a12 - a22]


def _rhs_terms(b11, b12, b21, b22):
    return [b11 + b22, b11, b12 - b22, b21 - b11, b22, b11 + b12, b21 + b22]


def _word_terms(terms, *blocks):
    lo, hi = [_low(u) for u in blocks], [_high(u) for u in blocks]
    out = []
    for a, b in zip(terms(*lo), terms(*hi)):
        plain = [u for u, l in zip(blocks, lo) if l is a]
        if plain:
            out.append(plain[0])
        else:
            y = jnp.concatenate([a, b], axis=1).astype(BF16).astype(F32)
            out.append((_words(y[:, :LANES]) >> 16) | _words(y[:, LANES:]))
    return out


def _combine(product, order=(5, 2, 4, 6, 0, 3, 1)):
    signs = ((1, 0, 0, 1), (0, 0, 1, -1), (0, 1, 0, 1), (1, 0, 1, 0),
             (-1, 1, 0, 0), (0, 0, 0, 1), (1, 0, 0, 0))
    plus, minus = [None] * 4, [None] * 4
    for i in order:
        m = product(i)
        for j, sign in enumerate(signs[i]):
            if sign > 0:
                plus[j] = m if plus[j] is None else plus[j] + m
            elif sign < 0:
                minus[j] = m
            if plus[j] is not None and minus[j] is not None:
                plus[j], minus[j] = plus[j] - minus[j], None
    c11, c12, c21, c22 = plus
    return [jnp.concatenate([y[r:r + 16] for r in range(0, top.shape[0], 16)
                             for y in (top, bot)], axis=0)
            for top, bot in ((c11, c21), (c12, c22))]


class _SideWork:
    def __init__(self, step, ndots, *lists):
        self.todo = sorted((((i + 0.5) / len(l), j, f)
                            for j, l in enumerate(lists) for i, f in enumerate(l)),
                           key=lambda e: e[:2])
        self.ndots, self.dots, self.last, self.done = ndots, 0, None, None
        self.never = jnp.full((8, LANES), step) < 0

    def dot(self, a, b):
        y = _dot(a, b)
        self.dots += 1
        self.last = y[0:8, 0:LANES]
        while self.todo and self.todo[0][0] * self.ndots <= self.dots:
            self.done = self.todo.pop(0)[2]()
        return y

    def pin(self, x):
        last = pltpu.bitcast(self.last, x.dtype)
        return jnp.concatenate([jnp.concatenate(
            [jnp.where(self.never, last, x[r:r + 8, c:c + LANES])
             for c in range(0, x.shape[1], LANES)], axis=1)
            for r in range(0, x.shape[0], 8)], axis=0)

    def after(self, x):
        if self.done is None:
            return x
        done, self.done = pltpu.bitcast(self.done[0:8], x.dtype), None
        return jnp.concatenate([jnp.where(self.never, done, x[:8]), x[8:]], axis=0)


def _project_b(hbm, xa_t, c_t, w_pair, wob_t, qb_p, kvb, sem, last_copy,
               xa, c, w_raw, xb, xb_t, wqkv, wqkv_t, wob, wob_tmp, qb, tr_tmp):
    xa_hbm, c_hbm, wq_hbm, wk_hbm, wv_hbm, xb_hbm, wqkv_hbm, wob_hbm = hbm
    rr = WROWS // NBM

    def xb_copy(i):
        rows = _ds(i * BM, BM, BM)
        return pltpu.make_async_copy(xb_hbm.at[rows], xb.at[rows], sem.at[i])

    wq_copies = [pltpu.make_async_copy(
        wqkv_hbm.at[:, j * M // 2:(j + 1) * M // 2],
        wqkv.at[:, j * M // 2:(j + 1) * M // 2], sem.at[NBM + j]) for j in range(2)]

    def wb_copies(i):
        rows = _ds(i * (M // 2), M // 2, M // 2)
        return [
            pltpu.make_async_copy(wqkv_hbm.at[rows, M:3 * M], wqkv.at[rows, M:3 * M],
                                  sem.at[NBM + 2 + i]),
            pltpu.make_async_copy(wob_hbm.at[rows], wob.at[rows], sem.at[NBM + 4 + i])]

    def a_copies(i, w_src):
        rows, first = _ds(i * BM, BM, BM), NBM + 6 + 3 * i
        return [
            pltpu.make_async_copy(w_src, w_raw.at[i], sem.at[first]),
            pltpu.make_async_copy(xa_hbm.at[rows], xa.at[rows], sem.at[first + 1]),
            pltpu.make_async_copy(c_hbm.at[rows], c.at[rows], sem.at[first + 2])]

    w_srcs = [w.at[r * H:(r + rr) * H]
              for w, n in ((wq_hbm, M), (wk_hbm, DC), (wv_hbm, DC))
              for r in range(0, n, rr)]
    copies = ([wq_copies[0]] + [xb_copy(i) for i in range(NBM)] + [wq_copies[1]] +
              wb_copies(0) + wb_copies(1))
    for i, src in enumerate(w_srcs):
        copies += a_copies(i, src)
    for cp in copies + [last_copy]:
        cp.start()

    def row_terms(src, dst, row0, t, pin=lambda u: u):
        top = _words(src[_ds(row0, 16, 16), t:t + 2 * LANES])
        bot = _words(src[_ds(row0 + 16, 16, 16), t:t + 2 * LANES])
        terms = _word_terms(_lhs_terms, pin(top[:, :LANES]), top[:, LANES:],
                            bot[:, :LANES], pin(bot[:, LANES:]))
        for i, u in enumerate(terms):
            dst[i, _ds(row0 // 4, 8, 8), t // 2:t // 2 + LANES] = u
        return terms

    def weight_terms(left, right):
        def blocks(u, odd):
            return jnp.concatenate(
                [u[r:r + 64] for r in range(64 * odd, u.shape[0], 128)], axis=0)
        return _word_terms(_rhs_terms, blocks(left, 0), blocks(right, 0),
                           blocks(left, 1), blocks(right, 1))

    def to_d_major(load, store, pin):
        def scatter(t):
            u = _words(load(t))
            ut = jnp.concatenate([pin(u[:8]), u[8:]], axis=0).T
            for j in range(LANES // DB):
                tr_tmp[pl.ds(4 * t + j, DB, stride=BPITCH), :] = ut[j * DB:(j + 1) * DB]

        def gather(t):
            store(t, jnp.concatenate(
                [tr_tmp[pl.ds((4 * t + j) * BPITCH, H), :] for j in range(4)], axis=0).T)

        return ([lambda t=t: scatter(t) for t in range(NTILE)] +
                [lambda t=t: gather(t) for t in range(NTILE)])

    def project_pair(side, weight, store):
        for g in range(NBM):
            ys = _combine(lambda i: side.dot(
                _bf16(xb_t[i, g * 64:(g + 1) * 64, :]), _bf16(weight(i))))
            for j, y in enumerate(ys):
                store(j, g * BM, y)

    for t in range(2 * NTILE):
        kvb[t, 0:HALO, :] = jnp.zeros((HALO, LANES), F32)
    wq_copies[0].wait()
    for p in range(2):
        w = _words(wqkv[:, p * 2 * LANES:(p + 1) * 2 * LANES])
        for i, u in enumerate(weight_terms(w[:, :LANES], w[:, LANES:])):
            wqkv_t[NTILE + p, i] = u

    def q_rows_step(i, carry):
        xb_copy(i).wait()
        terms = [[row_terms(xb, xb_t, i * BM + r, t) for t in range(0, M, 2 * LANES)]
                 for r in range(0, BM, 32)]
        terms = [jnp.concatenate(
            [jnp.concatenate([u[k] for u in row], axis=1) for row in terms], axis=0)
            for k in range(7)]
        orders = ([(2, 3, 4, 6, 0, 1, 5)], [])
        for p in range(2):
            ys = _combine(
                lambda k: _dot(_bf16(terms[k]), _bf16(wqkv_t[NTILE + p, k])), *orders[p])
            for j, y in enumerate(ys):
                qb[2 * p + j, _ds(i * BM, BM, BM), :] = y.astype(BF16)
        return carry

    lax.fori_loop(0, NBM, q_rows_step, 0)
    wq_copies[1].wait()

    def q_cols_step(i, carry):
        for cp in wb_copies(i):
            cp.wait()

        def permute_w(part, r):
            held = []

            def store(t, v):
                held.append(v)
                if t % 2:
                    for k, u in enumerate(weight_terms(*held[-2:])):
                        wqkv_t[(part * NTILE + t) // 2, k, _ds(r // 4, 64, 64), :] = u

            c0 = (1 + part) * M
            return to_d_major(
                lambda t: wqkv[_ds(r, BM, BM), c0 + t * LANES:c0 + (t + 1) * LANES],
                store, lambda u: side.pin(u))

        def scatter_wob(h):
            y = side.pin(wob[_ds(h * DB, DB, DB), :].astype(F32))
            for t in range(NTILE):
                wob_tmp[t, pl.ds(h, DB, stride=BPITCH), :] = y[:, t * LANES:(t + 1) * LANES]

        def store_q(j, r, y):
            qb[4 + 2 * i + j, r:r + BM, :] = y.astype(BF16)

        side = _SideWork(
            i, 7 * NBM - 4,
            [f for part in range(2) for r in (0, BM)
             for f in permute_w(part, i * 2 * BM + r)],
            [lambda j=j: scatter_wob(i * (H // 2) + j) for j in range(H // 2)])
        w = _words(wqkv[:, _ds(M // 2 + i * 2 * LANES, 2 * LANES, 2 * LANES)])
        w = weight_terms(w[:, :LANES], w[:, LANES:])
        project_pair(side, lambda k: w[k], store_q)
        return carry

    lax.fori_loop(0, 2, q_cols_step, 0)

    def kv_step(i, carry):
        for cp in a_copies(i, w_srcs[0]):
            cp.wait()

        def store_kv(j, r, y):
            kvb[2 * i + j, HALO + r:HALO + r + BM, :] = y

        def store_q(t, v):
            qb_p[t, _ds(i * LANES, LANES, LANES), :] = v

        def split_pairs(r):
            v = side.pin(_words(w_raw[i, r * H:(r + 4) * H, :]))
            for m in range(4):
                w_pair[pl.ds(i * rr + r + m, H // 2, stride=WPITCH), :] = (
                    v[m * H // 2:(m + 1) * H // 2])

        def wob_terms(d, n):
            blocks = [side.pin(wob_tmp[t, pl.ds(e * BPITCH, H), :])
                      for e in (d, d + DB // 2) for t in (2 * n, 2 * n + 1)]
            for k, y in enumerate(_rhs_terms(*blocks)):
                wob_t[k, _ds(d * H, H, H), n * LANES:(n + 1) * LANES] = y.astype(BF16)

        side = _SideWork(
            i, 7 * NBM - 4,
            [lambda r=r: split_pairs(r) for r in range(0, rr, 4)],
            to_d_major(lambda t: qb[t, _ds(i * BM, BM, BM), :], store_q,
                       lambda u: side.pin(u)),
            [lambda j=j, n=n: wob_terms(2 * i + j, n)
             for j in range(2) for n in range(NTILE // 2)],
            [lambda r=r, t=t, a=a: row_terms(*a, i * BM + r, t, side.pin)
             for r in range(0, BM, 32) for a in ((xa, xa_t), (c, c_t))
             for t in range(0, a[0].shape[1], 2 * LANES)])
        project_pair(side, lambda k: wqkv_t[i, k], store_kv)
        return carry

    lax.fori_loop(0, NBM, kv_step, 0)


def _attend_a(xa_t, c_t, w_pair, woa, ctx_t, woa_t, ks, vs):
    q_scale = D ** -0.5 * LOG2E

    def pair_step(pair, carry):
        def weight_terms(row0, n):
            top, bot = [jnp.concatenate(
                [w_pair[pl.ds(pair * WPITCH + row0 + r, LANES), :]
                 for r in range(odd * LANES, n, 2 * LANES)], axis=0) for odd in (0, 1)]
            return _rhs_terms(_low(top), _high(top), _low(bot), _high(bot))

        def out_weight_terms(r, n):
            top, bot = [_words(woa[_ds((2 * pair + j) * D + r, 16, 16),
                                   2 * n * LANES:2 * (n + 1) * LANES]) for j in range(2)]
            for i, u in enumerate(_word_terms(
                    _rhs_terms, side.pin(top[:, :LANES]), top[:, LANES:],
                    bot[:, :LANES], side.pin(bot[:, LANES:]))):
                woa_t[n, i, _ds((pair * D + r) // 2, 8, 8), :] = u

        side = _SideWork(pair, 28, [lambda r=r, n=n: out_weight_terms(r, n)
                                    for r in range(0, D, 16) for n in range(NTILE // 2)])
        causal = (lax.broadcasted_iota(jnp.int32, (LANES, LANES), 1) <=
                  lax.broadcasted_iota(jnp.int32, (LANES, LANES), 0))
        never = jnp.full((LANES, LANES), pair) < 0
        wkv = [jnp.concatenate([a, b], axis=1).astype(BF16)
               for a, b in zip(weight_terms(M, DC), weight_terms(M + DC, DC))]
        wq = [a.astype(BF16) for a in weight_terms(0, M)]
        q, ctx, finished = {}, {}, []

        def project_kv(g):
            kv = _combine(
                lambda i: _dot(_bf16(c_t[i, g * 64:(g + 1) * 64, :]), wkv[i]),
                *([] if g else [(4, 1, 2, 3, 6, 0, 5)]))
            for j in range(2):
                ks[j, g * BM:(g + 1) * BM, :] = kv[j][:, :D].astype(BF16)
                vs[j, g * BM:(g + 1) * BM, :] = kv[j][:, D:].astype(BF16)

        def project_q(g):
            ys = _combine(
                lambda i: side.dot(_bf16(xa_t[i, g * 64:(g + 1) * 64, :]), wq[i]))
            for j, y in enumerate(ys):
                q[j, 2 * g] = y[:LANES] * q_scale
                q[j, 2 * g + 1] = y[LANES:] * q_scale

        def scores(j, a):
            x = q[j, a]
            if len(finished) > 48:
                old, finished[:] = finished[:-48], finished[-48:]
                x = jnp.concatenate(
                    [x[:-8], jnp.where(never[:8], _fold(jnp.maximum, old), x[-8:])], axis=0)
            s = _dot_nt(x.astype(BF16), ks[j, 0:(a + 1) * LANES, :])
            s = [s[:, t * LANES:(t + 1) * LANES] for t in range(a + 1)]
            s[a] = jnp.where(causal, s[a], -1e30)
            return s

        def attend(j, a, s):
            m = jnp.max(_fold(jnp.maximum, s), axis=1, keepdims=True)
            p = [jnp.exp2(x - m) for x in s]
            total = _fold(jnp.add, p)
            if a:
                p[a] = jnp.where(never, total, p[a])
            o = _dot(jnp.concatenate(p, axis=1).astype(BF16), vs[j, 0:(a + 1) * LANES, :])
            ctx[j, a] = o * _recip(jnp.sum(total, axis=1, keepdims=True))
            finished.extend(ctx[j, a][r:r + 8] for r in range(0, LANES, 8))
            if j:
                for r in range(0, LANES, 32):
                    terms = _lhs_terms(ctx[0, a][r:r + 16], ctx[1, a][r:r + 16],
                                       ctx[0, a][r + 16:r + 32], ctx[1, a][r + 16:r + 32])
                    dst = (a * LANES + r) // 2
                    for i, y in enumerate(terms):
                        ctx_t[i, pair, dst:dst + 16, :] = y.astype(BF16)

        strips = [(j, a) for group in STRIPS for j in range(2) for a in group]
        kv_done, waiting = 0, None
        for n, (j, a) in enumerate(strips):
            while kv_done < NBM and (
                    kv_done <= n or any(b // 2 >= kv_done for _, b in strips[:n + 2])):
                project_kv(kv_done)
                kv_done += 1
            for key in strips[n:n + 4]:
                if key not in q:
                    project_q(key[1] // 2)
            s = scores(j, a)
            if waiting:
                attend(*waiting)
            waiting = (j, a, s)
        attend(*waiting)
        assert not side.todo
        return carry

    lax.fori_loop(0, H // 2, pair_step, 0)


def _project_out(out_hbm, ctx_t, woa_t, wob_t, qb_p, kvb, sem, att_t, oa_buf, ob_buf):
    b_scale = DB ** -0.5 * LOG2E
    nb = NTILE // 2

    def out_copies(i, slot):
        return [pltpu.make_async_copy(
            oa_buf.at[slot],
            out_hbm.at[_ds(i // 2 * 2 * BM, 2 * BM, BM),
                       _ds(slot * (M // 2), M // 2, M // 2)],
            sem.at[(1 + nb) * slot])] + [pltpu.make_async_copy(
                ob_buf.at[n, slot],
                out_hbm.at[_ds(i * BM, BM, BM),
                           M + 2 * n * LANES:M + 2 * (n + 1) * LANES],
                sem.at[(1 + nb) * slot + 1 + n]) for n in range(nb)]

    def window_attention(r0, a, held):
        q = [_bf16(qb_p[t, _ds((r0 + a) // 2, 8, 8), :]).astype(F32) for t in range(NTILE)]
        src = [pl.ds(r0 + HALO + a - DIL * w, 16) for w in range(WIN)]
        logits = []
        for w in range(WIN):
            l = _fold(jnp.add, [q[t] * kvb[t, src[w], :] for t in range(NTILE)])
            l = l + pltpu.roll(l, 2 * H, 1)
            l = (l + pltpu.roll(l, H, 1)) * b_scale
            if DIL * w > a:
                pos = r0 + a + lax.broadcasted_iota(jnp.int32, (16, LANES), 0)
                l = jnp.where(pos >= DIL * w, l, -1e30)
            logits.append(l)
        m = _fold(jnp.maximum, logits)
        e = [jnp.exp2(l - m) for l in logits]
        inv = _recip(_fold(jnp.add, e))
        e = [x * inv for x in e]
        o = [_fold(jnp.add, [e[w] * kvb[NTILE + t, src[w], :] for w in range(WIN)])
             for t in range(NTILE)]
        held.append(o)
        if a % 32:
            blocks = [jnp.concatenate(x, axis=1)
                      for y in held[-2:] for x in (y[:nb], y[nb:])]
            for i, y in enumerate(_lhs_terms(*blocks)):
                att_t[i, a // 32 * 16:a // 32 * 16 + 16, :] = y.astype(BF16)
        return o[-1]

    def out_step(i, carry):
        slot = i % 2
        r0 = pl.multiple_of(i * BM, BM)

        @pl.when(i >= 2)
        def _():
            for cp in out_copies(i - 2, slot):
                cp.wait()

        held = []
        side = _SideWork(i, 50, [lambda a=a: window_attention(r0, a, held)
                                 for a in range(0, BM, 16)])
        rows = _ds(i // 2 * BM, BM, BM)

        def product(n, k):
            y = None
            for p in range(0, H // 2, 4):
                part = side.dot(
                    jnp.concatenate([ctx_t[k, p + j, rows, :] for j in range(4)], axis=1),
                    _bf16(side.after(
                        woa_t[2 * slot + n, k, p * D // 2:(p + 4) * D // 2, :])))
                y = part if y is None else y + part
            return y

        for n in range(2):
            for j, y in enumerate(_combine(lambda k: product(n, k))):
                oa_buf[slot, :, (2 * n + j) * LANES:(2 * n + j + 1) * LANES] = y.astype(BF16)
        assert not side.todo
        copies = out_copies(i, slot)
        copies[0].start()
        for n in range(nb):
            ys = _combine(lambda k: _dot(att_t[k], wob_t[k, :, n * LANES:(n + 1) * LANES]))
            ob_buf[n, slot] = jnp.concatenate(ys, axis=1).astype(BF16)
            copies[1 + n].start()
        return carry

    lax.fori_loop(0, NBM, out_step, 0)
    for i in (NBM - 2, NBM - 1):
        for cp in out_copies(i, i % 2):
            cp.wait()


def _kernel(xa_hbm, c_hbm, wq_hbm, wk_hbm, wv_hbm, woa_hbm, xb_hbm, wqkv_hbm, wob_hbm,
            out_hbm, xa_t, c_t, w_pair, woa, wob_t, qb_p, kvb, in_sem, out_sem):
    vmem = pltpu.VMEM
    woa_copy = pltpu.make_async_copy(woa_hbm, woa, in_sem.at[4 * NBM + 6])
    tmp_rows = (DB + 2) * H
    pl.run_scoped(
        lambda *bufs: _project_b(
            (xa_hbm, c_hbm, wq_hbm, wk_hbm, wv_hbm, xb_hbm, wqkv_hbm, wob_hbm),
            xa_t, c_t, w_pair, wob_t, qb_p, kvb, in_sem, woa_copy, *bufs),
        vmem((S, M), BF16),
        vmem((S, DC), BF16),
        vmem((NBM, WROWS // NBM * H, D), BF16),
        vmem((S, M), BF16),
        vmem((7, S // 4, M // 2), U32),
        vmem((M, 3 * M), BF16),
        vmem((NTILE + 2, 7, M // 4, LANES), U32),
        vmem((M, M), BF16),
        vmem((NTILE, tmp_rows, LANES), F32),
        vmem((NTILE, S, LANES), BF16),
        vmem((tmp_rows, LANES), U32),
    )
    woa_copy.wait()

    def rest(ctx_t, woa_t, ks, vs, att_t, oa_buf, ob_buf):
        _attend_a(xa_t, c_t, w_pair, woa, ctx_t, woa_t, ks, vs)
        _project_out(out_hbm, ctx_t, woa_t, wob_t, qb_p, kvb, out_sem,
                     att_t, oa_buf, ob_buf)

    pl.run_scoped(
        rest,
        vmem((7, H // 2, S // 2, D), BF16),
        vmem((NTILE // 2, 7, H * D // 4, LANES), U32),
        vmem((2, S, D), BF16),
        vmem((2, S, D), BF16),
        vmem((7, BM // 2, M // 2), BF16),
        vmem((2, 2 * BM, M // 2), BF16),
        vmem((NTILE // 2, 2, BM, 2 * LANES), BF16),
    )


@jax.jit
def pallas_concat_heads__compressed_kv_cla__sliding_local_dilated__prompt_kernel(
    A_x: jax.Array,
    A_c_kv: jax.Array,
    A_w_q: jax.Array,
    A_w_uk: jax.Array,
    A_w_uv: jax.Array,
    A_w_o: jax.Array,
    B_x: jax.Array,
    B_wqkv: jax.Array,
    B_wo: jax.Array,
):
    vmem = pltpu.VMEM
    out = pl.pallas_call(
        _kernel,
        out_shape=jax.ShapeDtypeStruct((S, 2 * M), BF16),
        in_specs=[pl.BlockSpec(memory_space=pl.ANY)] * 9,
        out_specs=pl.BlockSpec(memory_space=pl.ANY),
        scratch_shapes=[
            vmem((7, S // 4, M // 2), U32),
            vmem((7, S // 4, DC // 2), U32),
            vmem(((H // 2 + 1) * WROWS + 32, D), U32),
            vmem((H * D, M), BF16),
            vmem((7, M // 2, M // 2), BF16),
            vmem((NTILE, S // 2, LANES), U32),
            vmem((2 * NTILE, HALO + S, LANES), F32),
            pltpu.SemaphoreType.DMA((4 * NBM + 7,)),
            pltpu.SemaphoreType.DMA((2 + NTILE,)),
        ],
        compiler_params=pltpu.CompilerParams(vmem_limit_bytes=126 * 2**20),
        name="fused_attn",
    )(
        A_x.reshape(S, M), A_c_kv.reshape(S, DC), A_w_q.reshape(M * H, D),
        A_w_uk.reshape(DC * H, D), A_w_uv.reshape(DC * H, D),
        A_w_o.reshape(H * D, M), B_x.reshape(S, M), B_wqkv, B_wo,
    )
    return out.reshape(1, S, 2 * M)
```

```python
import math

import jax
import jax.numpy as jnp
import numpy as np
from jax import lax
import jax.experimental.pallas as pl
import jax.experimental.pallas.tpu as pltpu

S = 2048
M = 1024
DC = 512
H = 32
D = 128
DB = 32
WIN, DIL = 8, 2
HALO = 16

LANES = 128
NTILE = M // LANES
BM = 256
NBM = S // BM
WROWS = M + 2 * DC
WPITCH = WROWS + 1
BPITCH = H + 1
STRIPS = ((0, 1), (2, 3), (5, 4), (8, 9), (10, 11), (12, 13), (15, 14), (6, 7))

LOG2E = math.log2(math.e)
BF16 = jnp.bfloat16
F32 = jnp.float32
U32 = jnp.uint32


def _dot(a, b):
    return jnp.dot(a, b, preferred_element_type=F32)


def _dot_nt(a, b):
    return lax.dot_general(a, b, (((1,), (1,)), ((), ())),
                           preferred_element_type=F32)


def _recip(x):
    r = pltpu.reciprocal(x, approx=True)
    return r * (2.0 - x * r)


def _fold(op, xs):
    y = xs[0]
    for x in xs[1:]:
        y = op(y, x)
    return y


def _ds(start, size, align):
    if not isinstance(start, int):
        start = pl.multiple_of(start, align)
    return pl.ds(start, size)


def _words(x):
    return pltpu.bitcast(x, U32)


def _bf16(u):
    return pltpu.bitcast(u, BF16)


def _low(u):
    return pltpu.bitcast(u << 16, F32)


def _high(u):
    return pltpu.bitcast(u & np.uint32(0xFFFF0000), F32)


def _lhs_terms(a11, a12, a21, a22):
    return [a11 + a22, a21 + a22, a11, a22, a11 + a12, a21 - a11, a12 - a22]


def _rhs_terms(b11, b12, b21, b22):
    return [b11 + b22, b11, b12 - b22, b21 - b11, b22, b11 + b12, b21 + b22]


def _word_terms(terms, *blocks):
    lo, hi = [_low(u) for u in blocks], [_high(u) for u in blocks]
    out = []
    for a, b in zip(terms(*lo), terms(*hi)):
        plain = [u for u, l in zip(blocks, lo) if l is a]
        if plain:
            out.append(plain[0])
        else:
            y = jnp.concatenate([a, b], axis=1).astype(BF16).astype(F32)
            out.append((_words(y[:, :LANES]) >> 16) | _words(y[:, LANES:]))
    return out


def _combine(product, order=(5, 2, 4, 6, 0, 3, 1)):
    signs = ((1, 0, 0, 1), (0, 0, 1, -1), (0, 1, 0, 1), (1, 0, 1, 0),
             (-1, 1, 0, 0), (0, 0, 0, 1), (1, 0, 0, 0))
    plus, minus = [None] * 4, [None] * 4
    for i in order:
        m = product(i)
        for j, sign in enumerate(signs[i]):
            if sign > 0:
                plus[j] = m if plus[j] is None else plus[j] + m
            elif sign < 0:
                minus[j] = m
            if plus[j] is not None and minus[j] is not None:
                plus[j], minus[j] = plus[j] - minus[j], None
    c11, c12, c21, c22 = plus
    return [jnp.concatenate([y[r:r + 16] for r in range(0, top.shape[0], 16)
                             for y in (top, bot)], axis=0)
            for top, bot in ((c11, c21), (c12, c22))]


class _SideWork:
    def __init__(self, step, ndots, *lists):
        self.todo = sorted((((i + 0.5) / len(l), j, f)
                            for j, l in enumerate(lists) for i, f in enumerate(l)),
                           key=lambda e: e[:2])
        self.ndots, self.dots, self.last, self.done = ndots, 0, None, None
        self.never = jnp.full((8, LANES), step) < 0

    def dot(self, a, b):
        y = _dot(a, b)
        self.dots += 1
        self.last = y[0:8, 0:LANES]
        while self.todo and self.todo[0][0] * self.ndots <= self.dots:
            self.done = self.todo.pop(0)[2]()
        return y

    def pin(self, x):
        last = pltpu.bitcast(self.last, x.dtype)
        return jnp.concatenate([jnp.concatenate(
            [jnp.where(self.never, last, x[r:r + 8, c:c + LANES])
             for c in range(0, x.shape[1], LANES)], axis=1)
            for r in range(0, x.shape[0], 8)], axis=0)

    def after(self, x):
        if self.done is None:
            return x
        done, self.done = pltpu.bitcast(self.done[0:8], x.dtype), None
        return jnp.concatenate([jnp.where(self.never, done, x[:8]), x[8:]], axis=0)


def _project_b(hbm, xa_t, c_t, w_pair, wob_t, qb_p, kvb, sem, last_copy,
               xa, c, w_raw, xb, xb_t, wqkv, wqkv_t, wob, wob_tmp, qb, tr_tmp):
    xa_hbm, c_hbm, wq_hbm, wk_hbm, wv_hbm, xb_hbm, wqkv_hbm, wob_hbm = hbm
    rr = WROWS // NBM

    def xb_copy(i):
        rows = _ds(i * BM, BM, BM)
        return pltpu.make_async_copy(xb_hbm.at[rows], xb.at[rows], sem.at[i])

    wq_copies = [pltpu.make_async_copy(
        wqkv_hbm.at[:, c0:c1], wqkv.at[:, c0:c1], sem.at[j]) for j, c0, c1 in (
            (NBM, 0, M // 4), (NBM + 1, M // 4, M // 2), (NBM + 2, M // 2, M))]

    def wb_copies(i):
        rows, done = _ds(i * (M // 2), M // 2, M // 2), sem.at[NBM + 3 + i]
        return [
            pltpu.make_async_copy(wqkv_hbm.at[rows, M:3 * M], wqkv.at[rows, M:3 * M], done),
            pltpu.make_async_copy(wob_hbm.at[rows], wob.at[rows], done)]

    def a_copies(i, w_src):
        rows, done = _ds(i * BM, BM, BM), sem.at[NBM + 5 + i]
        return [pltpu.make_async_copy(w_src, w_raw.at[i], done),
                pltpu.make_async_copy(xa_hbm.at[rows], xa.at[rows], done),
                pltpu.make_async_copy(c_hbm.at[rows], c.at[rows], done)]

    w_srcs = [w.at[r * H:(r + rr) * H]
              for w, n in ((wq_hbm, M), (wk_hbm, DC), (wv_hbm, DC))
              for r in range(0, n, rr)]
    copies = ([wq_copies[0], xb_copy(0), wq_copies[1]] +
              [xb_copy(i) for i in range(1, NBM)] + [wq_copies[2]] +
              wb_copies(0) + wb_copies(1))
    for i, src in enumerate(w_srcs):
        copies += a_copies(i, src)
    for cp in copies + [last_copy]:
        cp.start()

    def row_terms(src, dst, row0, t, pin=lambda u: u):
        top = _words(src[_ds(row0, 16, 16), t:t + 2 * LANES])
        bot = _words(src[_ds(row0 + 16, 16, 16), t:t + 2 * LANES])
        terms = _word_terms(_lhs_terms, pin(top[:, :LANES]), top[:, LANES:],
                            bot[:, :LANES], pin(bot[:, LANES:]))
        for i, u in enumerate(terms):
            dst[i, _ds(row0 // 4, 8, 8), t // 2:t // 2 + LANES] = u
        return terms

    def weight_terms(left, right):
        def blocks(u, odd):
            return jnp.concatenate(
                [u[r:r + 64] for r in range(64 * odd, u.shape[0], 128)], axis=0)
        return _word_terms(_rhs_terms, blocks(left, 0), blocks(right, 0),
                           blocks(left, 1), blocks(right, 1))

    def to_d_major(load, store, pin):
        def scatter(t):
            u = _words(load(t))
            ut = jnp.concatenate([pin(u[:8]), u[8:]], axis=0).T
            for j in range(LANES // DB):
                tr_tmp[pl.ds(4 * t + j, DB, stride=BPITCH), :] = ut[j * DB:(j + 1) * DB]

        def gather(t):
            store(t, jnp.concatenate(
                [tr_tmp[pl.ds((4 * t + j) * BPITCH, H), :] for j in range(4)], axis=0).T)

        return ([lambda t=t: scatter(t) for t in range(NTILE)] +
                [lambda t=t: gather(t) for t in range(NTILE)])

    def project_pair(side, weight, store):
        for g in range(NBM):
            ys = _combine(lambda i: side.dot(
                _bf16(xb_t[i, g * 64:(g + 1) * 64, :]), _bf16(weight(i))),
                (4, 2, 5, 6, 0, 3, 1))
            for j, y in enumerate(ys):
                store(j, g * BM, y)

    for t in range(2 * NTILE):
        kvb[t, 0:HALO, :] = jnp.zeros((HALO, LANES), F32)

    def first_weight_terms(p):
        wq_copies[p].wait()
        w = _words(wqkv[:, p * 2 * LANES:(p + 1) * 2 * LANES])
        for i, u in enumerate(weight_terms(w[:, :LANES], w[:, LANES:])):
            wqkv_t[NTILE + p, i] = u

    def q_rows_step(i, carry):
        xb_copy(i).wait()
        terms = [[row_terms(xb, xb_t, i * BM + r, t) for t in range(0, M, 2 * LANES)]
                 for r in range(0, BM, 32)]
        terms = [jnp.concatenate(
            [jnp.concatenate([u[k] for u in row], axis=1) for row in terms], axis=0)
            for k in range(7)]
        orders = ([(2, 3, 4, 6, 0, 1, 5)], [(4, 1, 2, 3, 6, 0, 5)])
        for p in range(2):
            if p and isinstance(i, int):
                first_weight_terms(p)
            ys = _combine(
                lambda k: _dot(_bf16(terms[k]), _bf16(wqkv_t[NTILE + p, k])), *orders[p])
            for j, y in enumerate(ys):
                qb[2 * p + j, _ds(i * BM, BM, BM), :] = y.astype(BF16)
        return carry

    first_weight_terms(0)
    q_rows_step(0, 0)
    lax.fori_loop(1, NBM, q_rows_step, 0)
    wq_copies[2].wait()

    def q_cols_step(i, carry):
        for cp in wb_copies(i):
            cp.wait()

        def permute_w(part, r):
            held = []

            def store(t, v):
                held.append(v)
                if t % 2:
                    for k, u in enumerate(weight_terms(*held[-2:])):
                        wqkv_t[(part * NTILE + t) // 2, k, _ds(r // 4, 64, 64), :] = u

            c0 = (1 + part) * M
            return to_d_major(
                lambda t: wqkv[_ds(r, BM, BM), c0 + t * LANES:c0 + (t + 1) * LANES],
                store, lambda u: side.pin(u))

        def scatter_wob(h):
            y = side.pin(wob[_ds(h * DB, DB, DB), :].astype(F32))
            for t in range(NTILE):
                wob_tmp[t, pl.ds(h, DB, stride=BPITCH), :] = y[:, t * LANES:(t + 1) * LANES]

        def store_q(j, r, y):
            qb[4 + 2 * i + j, r:r + BM, :] = y.astype(BF16)

        side = _SideWork(
            i, 7 * NBM - 4,
            [f for part in range(2) for r in (0, BM)
             for f in permute_w(part, i * 2 * BM + r)],
            [lambda j=j: scatter_wob(i * (H // 2) + j) for j in range(H // 2)])
        w = _words(wqkv[:, _ds(M // 2 + i * 2 * LANES, 2 * LANES, 2 * LANES)])
        w = weight_terms(w[:, :LANES], w[:, LANES:])
        project_pair(side, lambda k: w[k], store_q)
        return carry

    lax.fori_loop(0, 2, q_cols_step, 0)

    def kv_step(i, carry):
        for cp in a_copies(i, w_srcs[0]):
            cp.wait()

        def store_kv(j, r, y):
            kvb[2 * i + j, HALO + r:HALO + r + BM, :] = y

        def store_q(t, v):
            qb_p[t, _ds(i * LANES, LANES, LANES), :] = v

        def split_pairs(r):
            v = side.pin(_words(w_raw[i, r * H:(r + 4) * H, :]))
            for m in range(4):
                w_pair[pl.ds(i * rr + r + m, H // 2, stride=WPITCH), :] = (
                    v[m * H // 2:(m + 1) * H // 2])

        def wob_terms(d, n):
            blocks = [side.pin(wob_tmp[t, pl.ds(e * BPITCH, H), :])
                      for e in (d, d + DB // 2) for t in (2 * n, 2 * n + 1)]
            for k, y in enumerate(_rhs_terms(*blocks)):
                wob_t[k, _ds(d * H, H, H), n * LANES:(n + 1) * LANES] = y.astype(BF16)

        side = _SideWork(
            i, 7 * NBM - 4,
            [lambda r=r: split_pairs(r) for r in range(0, rr, 4)],
            to_d_major(lambda t: qb[t, _ds(i * BM, BM, BM), :], store_q,
                       lambda u: side.pin(u)),
            [lambda j=j, n=n: wob_terms(2 * i + j, n)
             for j in range(2) for n in range(NTILE // 2)],
            [lambda r=r, t=t, a=a: row_terms(*a, i * BM + r, t, side.pin)
             for r in range(0, BM, 32) for a in ((xa, xa_t), (c, c_t))
             for t in range(0, a[0].shape[1], 2 * LANES)])
        project_pair(side, lambda k: wqkv_t[i, k], store_kv)
        return carry

    lax.fori_loop(0, NBM, kv_step, 0)


def _attend_a(xa_t, c_t, w_pair, woa, ctx_t, woa_t, ks, vs):
    q_scale = D ** -0.5 * LOG2E

    def pair_step(pair, carry):
        def weight_terms(row0, n):
            top, bot = [jnp.concatenate(
                [w_pair[pl.ds(pair * WPITCH + row0 + r, LANES), :]
                 for r in range(odd * LANES, n, 2 * LANES)], axis=0) for odd in (0, 1)]
            return _rhs_terms(_low(top), _high(top), _low(bot), _high(bot))

        def out_weight_terms(r, n):
            top, bot = [_words(woa[_ds((2 * pair + j) * D + r, 16, 16),
                                   2 * n * LANES:2 * (n + 1) * LANES]) for j in range(2)]
            for i, u in enumerate(_word_terms(
                    _rhs_terms, side.pin(top[:, :LANES]), top[:, LANES:],
                    bot[:, :LANES], side.pin(bot[:, LANES:]))):
                woa_t[n, i, _ds((pair * D + r) // 2, 8, 8), :] = u

        side = _SideWork(pair, 28, [lambda r=r, n=n: out_weight_terms(r, n)
                                    for r in range(0, D, 16) for n in range(NTILE // 2)])
        causal = (lax.broadcasted_iota(jnp.int32, (LANES, LANES), 1) <=
                  lax.broadcasted_iota(jnp.int32, (LANES, LANES), 0))
        never = jnp.full((LANES, LANES), pair) < 0
        wkv = [jnp.concatenate([a, b], axis=1).astype(BF16)
               for a, b in zip(weight_terms(M, DC), weight_terms(M + DC, DC))]
        wq = [a.astype(BF16) for a in weight_terms(0, M)]
        q, ctx, finished = {}, {}, []

        def project_kv(g):
            kv = _combine(
                lambda i: _dot(_bf16(c_t[i, g * 64:(g + 1) * 64, :]), wkv[i]),
                *([] if g else [(4, 1, 2, 3, 6, 0, 5)]))
            for j in range(2):
                ks[j, g * BM:(g + 1) * BM, :] = kv[j][:, :D].astype(BF16)
                vs[j, g * BM:(g + 1) * BM, :] = kv[j][:, D:].astype(BF16)

        def project_q(g):
            ys = _combine(
                lambda i: side.dot(_bf16(xa_t[i, g * 64:(g + 1) * 64, :]), wq[i]))
            for j, y in enumerate(ys):
                q[j, 2 * g] = y[:LANES] * q_scale
                q[j, 2 * g + 1] = y[LANES:] * q_scale

        def scores(j, a):
            x = q[j, a]
            if len(finished) > 48:
                old, finished[:] = finished[:-48], finished[-48:]
                x = jnp.concatenate(
                    [x[:-8], jnp.where(never[:8], _fold(jnp.maximum, old), x[-8:])], axis=0)
            s = _dot_nt(x.astype(BF16), ks[j, 0:(a + 1) * LANES, :])
            s = [s[:, t * LANES:(t + 1) * LANES] for t in range(a + 1)]
            s[a] = jnp.where(causal, s[a], -1e30)
            return s

        def attend(j, a, s):
            m = jnp.max(_fold(jnp.maximum, s), axis=1, keepdims=True)
            p = [jnp.exp2(x - m) for x in s]
            total = _fold(jnp.add, p)
            if a:
                p[a] = jnp.where(never, total, p[a])
            o = _dot(jnp.concatenate(p, axis=1).astype(BF16), vs[j, 0:(a + 1) * LANES, :])
            ctx[j, a] = o * _recip(jnp.sum(total, axis=1, keepdims=True))
            finished.extend(ctx[j, a][r:r + 8] for r in range(0, LANES, 8))
            if j:
                for r in range(0, LANES, 32):
                    terms = _lhs_terms(ctx[0, a][r:r + 16], ctx[1, a][r:r + 16],
                                       ctx[0, a][r + 16:r + 32], ctx[1, a][r + 16:r + 32])
                    dst = (a * LANES + r) // 2
                    for i, y in enumerate(terms):
                        ctx_t[i, pair, dst:dst + 16, :] = y.astype(BF16)

        strips = [(j, a) for group in STRIPS for j in range(2) for a in group]
        kv_done, waiting = 0, None
        for n, (j, a) in enumerate(strips):
            while kv_done < NBM and (
                    kv_done <= n or any(b // 2 >= kv_done for _, b in strips[:n + 2])):
                project_kv(kv_done)
                kv_done += 1
            for key in strips[n:n + 4]:
                if key not in q:
                    project_q(key[1] // 2)
            s = scores(j, a)
            if waiting:
                attend(*waiting)
            waiting = (j, a, s)
        attend(*waiting)
        assert not side.todo
        return carry

    lax.fori_loop(0, H // 2, pair_step, 0)


def _project_out(out_hbm, ctx_t, woa_t, wob_t, qb_p, kvb, sem, att_t, oa_buf, ob_buf):
    b_scale = DB ** -0.5 * LOG2E
    nb = NTILE // 2

    def out_copies(i, slot):
        return [pltpu.make_async_copy(
            oa_buf.at[slot],
            out_hbm.at[_ds(i // 2 * 2 * BM, 2 * BM, BM),
                       _ds(slot * (M // 2), M // 2, M // 2)],
            sem.at[slot])] + [pltpu.make_async_copy(
                ob_buf.at[n, slot],
                out_hbm.at[_ds(i * BM, BM, BM),
                           M + 2 * n * LANES:M + 2 * (n + 1) * LANES],
                sem.at[slot]) for n in range(nb)]

    def window_attention(r0, a, held):
        q = [_bf16(qb_p[t, _ds((r0 + a) // 2, 8, 8), :]).astype(F32) for t in range(NTILE)]
        src = [pl.ds(r0 + HALO + a - DIL * w, 16) for w in range(WIN)]
        logits = []
        for w in range(WIN):
            l = _fold(jnp.add, [q[t] * kvb[t, src[w], :] for t in range(NTILE)])
            l = l + pltpu.roll(l, 2 * H, 1)
            l = (l + pltpu.roll(l, H, 1)) * b_scale
            if DIL * w > a:
                pos = r0 + a + lax.broadcasted_iota(jnp.int32, (16, LANES), 0)
                l = jnp.where(pos >= DIL * w, l, -1e30)
            logits.append(l)
        m = _fold(jnp.maximum, logits)
        e = [jnp.exp2(l - m) for l in logits]
        inv = _recip(_fold(jnp.add, e))
        e = [x * inv for x in e]
        o = [_fold(jnp.add, [e[w] * kvb[NTILE + t, src[w], :] for w in range(WIN)])
             for t in range(NTILE)]
        held.append(o)
        if a % 32:
            blocks = [jnp.concatenate(x, axis=1)
                      for y in held[-2:] for x in (y[:nb], y[nb:])]
            for i, y in enumerate(_lhs_terms(*blocks)):
                att_t[i, a // 32 * 16:a // 32 * 16 + 16, :] = y.astype(BF16)
        return o[-1]

    def out_step(i, carry):
        slot = i % 2
        r0 = pl.multiple_of(i * BM, BM)

        @pl.when(i >= 2)
        def _():
            for cp in out_copies(i - 2, slot):
                cp.wait()

        held = []
        side = _SideWork(i, 50, [lambda a=a: window_attention(r0, a, held)
                                 for a in range(0, BM, 16)])
        rows = _ds(i // 2 * BM, BM, BM)

        def product(n, k):
            y = None
            for p in range(0, H // 2, 4):
                part = side.dot(
                    jnp.concatenate([ctx_t[k, p + j, rows, :] for j in range(4)], axis=1),
                    _bf16(side.after(
                        woa_t[2 * slot + n, k, p * D // 2:(p + 4) * D // 2, :])))
                y = part if y is None else y + part
            return y

        for n in range(2):
            for j, y in enumerate(_combine(lambda k: product(n, k))):
                oa_buf[slot, :, (2 * n + j) * LANES:(2 * n + j + 1) * LANES] = y.astype(BF16)
        assert not side.todo
        copies = out_copies(i, slot)
        copies[0].start()
        for n in range(nb):
            ys = _combine(lambda k: _dot(att_t[k], wob_t[k, :, n * LANES:(n + 1) * LANES]))
            ob_buf[n, slot] = jnp.concatenate(ys, axis=1).astype(BF16)
            copies[1 + n].start()
        return carry

    lax.fori_loop(0, NBM, out_step, 0)
    for i in (NBM - 2, NBM - 1):
        for cp in out_copies(i, i % 2):
            cp.wait()


def _kernel(xa_hbm, c_hbm, wq_hbm, wk_hbm, wv_hbm, woa_hbm, xb_hbm, wqkv_hbm, wob_hbm,
            out_hbm, xa_t, c_t, w_pair, woa, wob_t, qb_p, kvb, in_sem, out_sem):
    vmem = pltpu.VMEM
    woa_copy = pltpu.make_async_copy(woa_hbm, woa, in_sem.at[2 * NBM + 5])
    tmp_rows = (DB + 2) * H
    pl.run_scoped(
        lambda *bufs: _project_b(
            (xa_hbm, c_hbm, wq_hbm, wk_hbm, wv_hbm, xb_hbm, wqkv_hbm, wob_hbm),
            xa_t, c_t, w_pair, wob_t, qb_p, kvb, in_sem, woa_copy, *bufs),
        vmem((S, M), BF16),
        vmem((S, DC), BF16),
        vmem((NBM, WROWS // NBM * H, D), BF16),
        vmem((S, M), BF16),
        vmem((7, S // 4, M // 2), U32),
        vmem((M, 3 * M), BF16),
        vmem((NTILE + 2, 7, M // 4, LANES), U32),
        vmem((M, M), BF16),
        vmem((NTILE, tmp_rows, LANES), F32),
        vmem((NTILE, S, LANES), BF16),
        vmem((tmp_rows, LANES), U32),
    )
    woa_copy.wait()

    def rest(ctx_t, woa_t, ks, vs, att_t, oa_buf, ob_buf):
        _attend_a(xa_t, c_t, w_pair, woa, ctx_t, woa_t, ks, vs)
        _project_out(out_hbm, ctx_t, woa_t, wob_t, qb_p, kvb, out_sem,
                     att_t, oa_buf, ob_buf)

    pl.run_scoped(
        rest,
        vmem((7, H // 2, S // 2, D), BF16),
        vmem((NTILE // 2, 7, H * D // 4, LANES), U32),
        vmem((2, S, D), BF16),
        vmem((2, S, D), BF16),
        vmem((7, BM // 2, M // 2), BF16),
        vmem((2, 2 * BM, M // 2), BF16),
        vmem((NTILE // 2, 2, BM, 2 * LANES), BF16),
    )


@jax.jit
def pallas_concat_heads__compressed_kv_cla__sliding_local_dilated__prompt_kernel(
    A_x: jax.Array,
    A_c_kv: jax.Array,
    A_w_q: jax.Array,
    A_w_uk: jax.Array,
    A_w_uv: jax.Array,
    A_w_o: jax.Array,
    B_x: jax.Array,
    B_wqkv: jax.Array,
    B_wo: jax.Array,
):
    vmem = pltpu.VMEM
    out = pl.pallas_call(
        _kernel,
        out_shape=jax.ShapeDtypeStruct((S, 2 * M), BF16),
        in_specs=[pl.BlockSpec(memory_space=pl.ANY)] * 9,
        out_specs=pl.BlockSpec(memory_space=pl.ANY),
        scratch_shapes=[
            vmem((7, S // 4, M // 2), U32),
            vmem((7, S // 4, DC // 2), U32),
            vmem(((H // 2 + 1) * WROWS + 32, D), U32),
            vmem((H * D, M), BF16),
            vmem((7, M // 2, M // 2), BF16),
            vmem((NTILE, S // 2, LANES), U32),
            vmem((2 * NTILE, HALO + S, LANES), F32),
            pltpu.SemaphoreType.DMA((2 * NBM + 6,)),
            pltpu.SemaphoreType.DMA((2,)),
        ],
        compiler_params=pltpu.CompilerParams(vmem_limit_bytes=126 * 2**20),
        name="fused_attn",
    )(
        A_x.reshape(S, M), A_c_kv.reshape(S, DC), A_w_q.reshape(M * H, D),
        A_w_uk.reshape(DC * H, D), A_w_uv.reshape(DC * H, D),
        A_w_o.reshape(H * D, M), B_x.reshape(S, M), B_wqkv, B_wo,
    )
    return out.reshape(1, S, 2 * M)
```
